```python
import jax
import jax.numpy as jnp

def _softmax(x, axis=-1):
    return jax.nn.softmax(x, axis=axis)
def _gelu(x):
    return jax.nn.gelu(x, approximate=True)
def _silu(x):
    return jax.nn.silu(x)
def _sigmoid(x):
    return jax.nn.sigmoid(x)
def _layernorm(x, axis=-1, eps=1e-5):
    m = jnp.mean(x, axis=axis, keepdims=True)
    v = jnp.var(x, axis=axis, keepdims=True)
    return (x - m) / jnp.sqrt(v + eps)
def _scatter_add(tgt, idx, src, axis=0):
    return tgt.at[idx].add(src)
def _segment_sum(src, seg, n):
    return jax.ops.segment_sum(src, seg, n)
class _Rng:
    def __init__(self, key):
        self._k = key
    def _next(self):
        self._k, sub = jax.random.split(self._k)
        return sub
    def normal(self, shape):
        return jax.random.normal(self._next(), shape, dtype=jnp.bfloat16)
    def randint(self, lo, hi, shape):
        return jax.random.randint(self._next(), shape, lo, hi, dtype=jnp.int32)
    def uniform(self, shape, lo=0.0, hi=1.0):
        return jax.random.uniform(self._next(), shape, jnp.bfloat16, lo, hi)
    def permutation(self, n):
        return jax.random.permutation(self._next(), n)


kernel_name = 'standalone__seq2seq_rnn_t_joint__speech'

def setup_inputs():
    _rng = _Rng(jax.random.key(int.from_bytes(__import__("os").urandom(4), "little")))
    _w = (lambda a: (lambda t: t.astype(jnp.bfloat16) if jnp.issubdtype(t.dtype, jnp.floating) else t)(jnp.asarray(a)))
    B, T, D, K = 2, 16000, 256, 31
    U = 8
    sc = (1.0 / (K * D)) ** 0.5
    sd = (1.0 / D) ** 0.5
    return {
        "x": _w((lambda *s: _rng.normal(s) * 0.05)(B, T, D) * 0.5),
        "w1": _w((lambda *s: _rng.normal(s) * 0.05)(K, D, D) * sc),
        "w2": _w((lambda *s: _rng.normal(s) * 0.05)(K, D, D) * sc),
        "g": _w((lambda *s: _rng.normal(s) * 0.05)(B, U, D) * 0.5),
        "w_f": _w((lambda *s: _rng.normal(s) * 0.05)(D, D) * sd),
        "w_g": _w((lambda *s: _rng.normal(s) * 0.05)(D, D) * sd),
        "w_o": _w((lambda *s: _rng.normal(s) * 0.05)(D, D) * sd),
    }

def reference(x, w1, w2, g, w_f, w_g, w_o):
    B, T, D = x.shape
    K = w1.shape[0]
    pad = K // 2
    xp = jnp.pad(x, ((0,0),(pad,pad),(0,0)))
    h = jnp.zeros_like(x)
    for i in range(K):
        h = h + jnp.einsum("btc,cd->btd", xp[:, i:i+T, :], w1[i])
    h = _gelu(h)[:, ::2, :]
    T1 = h.shape[1]
    hp = jnp.pad(h, ((0,0),(pad,pad),(0,0)))
    f = jnp.zeros_like(h)
    for i in range(K):
        f = f + jnp.einsum("btc,cd->btd", hp[:, i:i+T1, :], w2[i])
    f = _gelu(f)[:, ::2, :]
    fe = jnp.einsum("btd,de->bte", f, w_f)
    ge = jnp.einsum("bud,de->bue", g, w_g)
    j = jnp.tanh(fe[:, :, None, :] + ge[:, None, :, :])
    return jnp.einsum("btud,dv->btuv", j, w_o)
```

```python
import functools
import jax
import jax.numpy as jnp
import numpy as np
import jax.experimental.pallas as pl
import jax.experimental.pallas.tpu as pltpu

B, T, D, K, U = 2, 16000, 256, 31, 8
T1, T2 = T // 2, T // 4
MT1 = 400
MT2 = 500
NT2 = T2 // MT2

_C0 = float(np.sqrt(2.0 / np.pi))
_C1 = 0.044715


def _gelu(x):
    return 0.5 * x * (1.0 + jnp.tanh(_C0 * (x + _C1 * (x * x * x))))


def _conv_tile(words_ref, t0, mt, w_ref):
    win = words_ref[pl.ds(t0, mt + 16), :]
    lo = pltpu.bitcast(win << 16, jnp.float32)
    hi = pltpu.bitcast(win & jnp.uint32(0xFFFF0000), jnp.float32)
    acc = jnp.dot(hi[0:mt].astype(jnp.bfloat16), w_ref[0], preferred_element_type=jnp.float32)
    for j in range(1, 16):
        lhs = jnp.concatenate([lo[j:j + mt], hi[j:j + mt]], axis=1).astype(jnp.bfloat16)
        rhs = w_ref[2 * j - 1:2 * j + 1].reshape(2 * D, D)
        acc = acc + jnp.dot(lhs, rhs, preferred_element_type=jnp.float32)
    return acc


def _kernel(x_hbm, w1_ref, w2_ref, g_ref, wf_ref, wg_ref, wo_ref, o_ref, xbuf, hbuf, sem):
    b = pl.program_id(0)
    i = pl.program_id(1)

    @pl.when(i == 0)
    def _():
        xbuf[pl.ds(0, 16), :] = jnp.zeros((16, D), jnp.bfloat16)
        xbuf[pl.ds(16 + T, 16), :] = jnp.zeros((16, D), jnp.bfloat16)
        cp = pltpu.make_async_copy(x_hbm.at[b], xbuf.at[pl.ds(16, T), :], sem)
        cp.start()
        cp.wait()
        hbuf[pl.ds(0, 16), :] = jnp.zeros((16, D), jnp.bfloat16)
        hbuf[pl.ds(16 + T1, 16), :] = jnp.zeros((16, D), jnp.bfloat16)
        xw = xbuf.bitcast(jnp.uint32)

        def body(n, c):
            t0 = pl.multiple_of(n * MT1, 8)
            acc = _conv_tile(xw, t0, MT1, w1_ref)
            hbuf[pl.ds(pl.multiple_of(16 + n * MT1, 16), MT1), :] = _gelu(acc).astype(jnp.bfloat16)
            return c
        jax.lax.fori_loop(0, T1 // MT1, body, 0)

    hw = hbuf.bitcast(jnp.uint32)
    SUB = 100 if False else MT2
    t0 = i * MT2
    acc = _conv_tile(hw, t0, MT2, w2_ref)
    f = _gelu(acc).astype(jnp.bfloat16)
    fe = jnp.dot(f, wf_ref[...], preferred_element_type=jnp.float32)
    ge = jnp.dot(g_ref[0], wg_ref[...], preferred_element_type=jnp.float32)
    j = jnp.tanh(fe[:, None, :] + ge[None, :, :]).reshape(MT2 * U, D).astype(jnp.bfloat16)
    o = jnp.dot(j, wo_ref[...], preferred_element_type=jnp.float32)
    o_ref[0] = o.reshape(MT2, U, D).astype(jnp.bfloat16)


@jax.jit
def pallas_standalone__seq2seq_rnn_t_joint__speech_kernel(x, w1, w2, g, w_f, w_g, w_o):
    return pl.pallas_call(
        _kernel,
        grid=(B, NT2),
        in_specs=[
            pl.BlockSpec(memory_space=pl.ANY),
            pl.BlockSpec((K, D, D), lambda b, i: (0, 0, 0)),
            pl.BlockSpec((K, D, D), lambda b, i: (0, 0, 0)),
            pl.BlockSpec((1, U, D), lambda b, i: (b, 0, 0)),
            pl.BlockSpec((D, D), lambda b, i: (0, 0)),
            pl.BlockSpec((D, D), lambda b, i: (0, 0)),
            pl.BlockSpec((D, D), lambda b, i: (0, 0)),
        ],
        out_specs=pl.BlockSpec((1, MT2, U, D), lambda b, i: (b, i, 0, 0)),
        out_shape=jax.ShapeDtypeStruct((B, T2, U, D), jnp.bfloat16),
        scratch_shapes=[
            pltpu.VMEM((T + 32, D), jnp.bfloat16),
            pltpu.VMEM((T1 + 32, D), jnp.bfloat16),
            pltpu.SemaphoreType.DMA,
        ],
        compiler_params=pltpu.CompilerParams(
            dimension_semantics=("arbitrary", "arbitrary"),
            vmem_limit_bytes=100 * 1024 * 1024,
        ),
        name="rnnt_base",
    )(x, w1, w2, g, w_f, w_g, w_o)
```

```python
import functools
import numpy as np
import jax
import jax.numpy as jnp
from jax import lax
import jax.experimental.pallas as pl
import jax.experimental.pallas.tpu as pltpu

B, T, D, K, U = 2, 16000, 256, 31, 8
H = D // 2
T1, T2 = T // 2, T // 4
N = 64
HOP = 46
NB1 = 176
NB2 = NB1 // 2
P1 = NB1 * HOP
P2 = NB2 * HOP
P3 = NB2 * HOP // 2
XR = 8 + B * P1 + 24
HR = 8 + B * P2 + 24
FR = B * P3
TT = 160
RS2 = float(np.sqrt(0.5))
HIMASK = np.uint32(0xFFFF0000)
OSCALE = 1.0 / (2 * N)
GC0 = float(np.sqrt(2.0 / np.pi))
GC1 = 0.044715


def _fft8(xr, xi):
    a0r, a0i = xr[0] + xr[4], xi[0] + xi[4]
    a1r, a1i = xr[0] - xr[4], xi[0] - xi[4]
    a2r, a2i = xr[2] + xr[6], xi[2] + xi[6]
    a3r, a3i = xr[2] - xr[6], xi[2] - xi[6]
    a4r, a4i = xr[1] + xr[5], xi[1] + xi[5]
    a5r, a5i = xr[1] - xr[5], xi[1] - xi[5]
    a6r, a6i = xr[3] + xr[7], xi[3] + xi[7]
    a7r, a7i = xr[3] - xr[7], xi[3] - xi[7]
    e0r, e0i = a0r + a2r, a0i + a2i
    e2r, e2i = a0r - a2r, a0i - a2i
    e1r, e1i = a1r + a3i, a1i - a3r
    e3r, e3i = a1r - a3i, a1i + a3r
    o0r, o0i = a4r + a6r, a4i + a6i
    o2r, o2i = a4r - a6r, a4i - a6i
    o1r, o1i = a5r + a7i, a5i - a7r
    o3r, o3i = a5r - a7i, a5i + a7r
    t1r, t1i = (o1r + o1i) * RS2, (o1i - o1r) * RS2
    u, v = (o3i - o3r) * RS2, (o3r + o3i) * RS2
    yr = [e0r + o0r, e1r + t1r, e2r + o2i, e3r + u, e0r - o0r, e1r - t1r, e2r - o2i, e3r - u]
    yi = [e0i + o0i, e1i + t1i, e2i - o2r, e3i - v, e0i - o0i, e1i - t1i, e2i + o2r, e3i + v]
    return yr, yi


def _ifft8(xr, xi):
    yi, yr = _fft8(xi, xr)
    return yr, yi


def _idft4(xr, xi):
    s02r, s02i = xr[0] + xr[2], xi[0] + xi[2]
    d02r, d02i = xr[0] - xr[2], xi[0] - xi[2]
    s13r, s13i = xr[1] + xr[3], xi[1] + xi[3]
    d13r, d13i = xr[1] - xr[3], xi[1] - xi[3]
    yr = [s02r + s13r, d02r - d13i, s02r - s13r, d02r + d13i]
    yi = [s02i + s13i, d02i + d13r, s02i - s13i, d02i - d13r]
    return yr, yi


def _tw(ar, ai, num, den):
    num = num % den
    if num == 0:
        return ar, ai
    if num * 4 == den:
        return -ai, ar
    if num * 2 == den:
        return -ar, -ai
    if num * 4 == 3 * den:
        return ai, -ar
    if (num * 8) % den == 0:
        q = num * 8 // den
        if q == 1:
            return (ar - ai) * RS2, (ar + ai) * RS2
        if q == 3:
            return (ar + ai) * (-RS2), (ar - ai) * RS2
        if q == 5:
            return (ai - ar) * RS2, (ar + ai) * (-RS2)
        return (ar + ai) * RS2, (ai - ar) * RS2
    c = float(np.cos(2 * np.pi * num / den))
    s = float(np.sin(2 * np.pi * num / den))
    return ar * c - ai * s, ar * s + ai * c


def _gelu_scaled(v):
    s = OSCALE
    t = v * v
    inner = v * (t * float(GC0 * GC1 * s * s * s) + float(GC0 * s))
    hv = v * float(0.5 * s)
    return hv + hv * jnp.tanh(inner)


def _lo(w):
    return pltpu.bitcast(w << 16, jnp.float32)


def _hi(w):
    return pltpu.bitcast(w & HIMASK, jnp.float32)


def _fwd_pass1(src, tr, ti):
    for n2 in range(8):
        xr, xi = [], []
        for n1 in range(8):
            w = src[pl.ds(8 * n1 + n2, 8, stride=HOP), :]
            xr.append(_lo(w))
            xi.append(_hi(w))
        ar, ai = _fft8(xr, xi)
        for k1 in range(8):
            br, bi = _tw(ar[k1], ai[k1], -n2 * k1, N)
            tr[k1, n2] = br
            ti[k1, n2] = bi


def _fwd_pass2(tar, tai, tbr, tbi, zbuf, row0, col, k1s=range(8)):
    for k1 in k1s:
        ya_r, ya_i = _fft8([tar[k1, n] for n in range(8)], [tai[k1, n] for n in range(8)])
        yb_r, yb_i = _fft8([tbr[k1, n] for n in range(8)], [tbi[k1, n] for n in range(8)])
        for k2 in range(8):
            k = k1 + 8 * k2
            r = jnp.concatenate([ya_r[k2], yb_r[k2]], axis=0)
            i = jnp.concatenate([ya_i[k2], yb_i[k2]], axis=0)
            cs = pl.ds(col * H, H)
            zbuf[0, k, pl.ds(row0, 16), cs] = (r + i).astype(jnp.bfloat16)
            zbuf[1, k, pl.ds(row0, 16), cs] = r.astype(jnp.bfloat16)
            zbuf[2, k, pl.ds(row0, 16), cs] = i.astype(jnp.bfloat16)


def _m_step(k, zbuf, wf, vr, vi):
    kn = (N - k) & (N - 1)
    l1 = jnp.concatenate([zbuf[0, k], zbuf[0, kn]], axis=1)
    l2 = jnp.concatenate([zbuf[2, k], zbuf[1, kn]], axis=1)
    l3 = jnp.concatenate([zbuf[1, k], zbuf[2, kn]], axis=1)
    g1 = jnp.dot(l1, wf[k, 0], preferred_element_type=jnp.float32)
    g2 = jnp.dot(l2, wf[k, 1], preferred_element_type=jnp.float32)
    g3 = jnp.dot(l3, wf[k, 2], preferred_element_type=jnp.float32)
    vr[k] = g1 - g2
    vi[k] = g1 - g3


def _inv_passA(vr, vi, row0, ur, ui):
    for k1 in range(8):
        xr = [vr[k1 + 8 * k2, pl.ds(row0, 8), :] for k2 in range(8)]
        xi = [vi[k1 + 8 * k2, pl.ds(row0, 8), :] for k2 in range(8)]
        ar, ai = _ifft8(xr, xi)
        for m2 in range(8):
            br, bi = _tw(ar[m2], ai[m2], m2 * k1, N)
            ur[m2, k1] = br
            ui[m2, k1] = bi


def _inv_passB(ur, ui, dst0, dst1):
    for q in range(4):
        ys = []
        for m2 in (2 * q, 2 * q + 1):
            yr, yi = _ifft8([ur[m2, k1] for k1 in range(8)], [ui[m2, k1] for k1 in range(8)])
            ys.append((yr, yi))
        for m1 in range(6):
            m = 8 * m1 + 2 * q
            if m >= HOP:
                continue
            for dst, part in ((dst0, 0), (dst1, 1)):
                a = _gelu_scaled(ys[0][part][m1])
                b = _gelu_scaled(ys[1][part][m1])
                dst[pl.ds(m // 2, 8, stride=HOP // 2), :] = pltpu.pack_elementwise(
                    [a, b], packed_dtype=jnp.bfloat16)


def _w_step(w_ref, slab, is_q, pbuf_r, pbuf_i, sr, si, wf, z3):
    rows = pl.ds(pl.multiple_of(slab * 16, 16), 16)
    c0, c1 = pl.ds(0, H), pl.ds(H, H)
    f32 = jnp.float32
    for j in range(16):
        vo0 = w_ref[2 * j, rows, c0].astype(f32)
        vo1 = w_ref[2 * j, rows, c1].astype(f32)
        if j == 0:
            pr, pi = (-vo1, vo0) if is_q else (vo1, -vo0)
        else:
            ve0 = w_ref[2 * j - 1, rows, c0].astype(f32)
            ve1 = w_ref[2 * j - 1, rows, c1].astype(f32)
            pr, pi = (ve0 - vo1, ve1 + vo0) if is_q else (ve0 + vo1, ve1 - vo0)
        pbuf_r[j] = pr
        pbuf_i[j] = pi
    pr_ = pbuf_r.at[pl.ds(z3, 16)]
    pi_ = pbuf_i.at[pl.ds(z3, 16)]
    sr_ = sr.at[pl.ds(z3, 4)]
    si_ = si.at[pl.ds(z3, 4)]
    off = (D if is_q else 0)
    orow = pl.ds(pl.multiple_of(slab * 16 + off, 16), 16)
    for r in range(4):
        for j2 in range(4):
            xr, xi = [], []
            for j1 in range(4):
                j = 4 * j1 + j2
                a, b = _tw(pr_[j], pi_[j], j * r, N)
                xr.append(a)
                xi.append(b)
            yr, yi = _idft4(xr, xi)
            for k1 in range(4):
                a, b = _tw(yr[k1], yi[k1], j2 * k1, 16)
                sr[r, k1, j2] = a
                si[r, k1, j2] = b
    for r in range(4):
        for k1 in range(4):
            yr, yi = _idft4([sr_[r, k1, j2] for j2 in range(4)], [si_[r, k1, j2] for j2 in range(4)])
            for k2 in range(4):
                k = 4 * (k1 + 4 * k2) + r
                if is_q:
                    m0, m1, m2 = yi[k2], yi[k2] - yr[k2], yi[k2] + yr[k2]
                else:
                    m0, m1, m2 = yr[k2], yr[k2] + yi[k2], yr[k2] - yi[k2]
                wf[k, 0, orow, :] = m0.astype(jnp.bfloat16)
                wf[k, 1, orow, :] = m1.astype(jnp.bfloat16)
                wf[k, 2, orow, :] = m2.astype(jnp.bfloat16)


def _w_transform(w_ref, wf, pbuf_r, pbuf_i, sr, si):
    def body(s, c):
        z = s >> 16
        _w_step(w_ref, s, False, pbuf_r, pbuf_i, sr, si, wf, z)
        _w_step(w_ref, s, True, pbuf_r, pbuf_i, sr, si, wf, z)
        return c
    lax.fori_loop(0, D // 16, body, 0)


def _conv_chunk(srcw, base_row, m_rows, zbuf, wf, vr, vi, tbufs, ubufs, dstw, dst_row):
    tar, tai, tbr, tbi = tbufs
    ur, ui = ubufs

    def fbody(g, c):
        z = g >> 16
        start = pl.multiple_of(base_row + g * (16 * HOP), 8)
        for col in range(2):
            sub = srcw.at[col, pl.ds(start, 16 * HOP + 32), :]
            _fwd_pass1(sub, tar, tai)
            _fwd_pass1(sub.at[pl.ds(8 * HOP, 8 * HOP + 32), :], tbr, tbi)
            row0 = pl.multiple_of(g * 16, 16)
            views = [t.at[pl.ds(z, 8)] for t in (tar, tai, tbr, tbi)]
            _fwd_pass2(*views, zbuf, row0, col)
        return c
    lax.fori_loop(0, m_rows // 16, fbody, 0)

    def mbody(k, c):
        _m_step(k, zbuf, wf, vr, vi)
        return c
    lax.fori_loop(0, N, mbody, 0)

    def ibody(g, c):
        z = g >> 16
        row0 = pl.multiple_of(g * 8, 8)
        _inv_passA(vr, vi, row0, ur, ui)
        d0 = pl.multiple_of(dst_row + g * (8 * HOP // 2), 8)
        n = 8 * HOP // 2
        _inv_passB(ur.at[pl.ds(z, 8)], ui.at[pl.ds(z, 8)],
                   dstw.at[0, pl.ds(d0, n), :], dstw.at[1, pl.ds(d0, n), :])
        return c
    lax.fori_loop(0, m_rows // 8, ibody, 0)


def _kernel(x_hbm, w1_hbm, w2_hbm, g_ref, wf_ref, wg_ref, wo_ref, o_hbm,
            xbuf, hbuf, fbuf, wraw, wfreq, zbuf, vr, vi,
            t0, t1, t2, t3, ur, ui, pbr, pbi, sr, si, obuf, sems, osems):
    bf = jnp.bfloat16
    wcp = pltpu.make_async_copy(w1_hbm, wraw, sems.at[4])
    wcp.start()
    xcps = []
    for b in range(B):
        for c in range(2):
            cp = pltpu.make_async_copy(
                x_hbm.at[b, :, pl.ds(c * H, H)],
                xbuf.at[c, pl.ds(16 + b * 2 * P1, T), :], sems.at[b * 2 + c])
            cp.start()
            xcps.append(cp)
    for c in range(2):
        xbuf[c, pl.ds(0, 16), :] = jnp.zeros((16, H), bf)
        for b in range(B):
            n = 2 * P1 - T + (48 if b == B - 1 else 0)
            xbuf[c, pl.ds(16 + b * 2 * P1 + T, n), :] = jnp.zeros((n, H), bf)
        hbuf[c, pl.ds(0, 16), :] = jnp.zeros((16, H), bf)
        hbuf[c, pl.ds(16 + B * 2 * P2, 48), :] = jnp.zeros((48, H), bf)
    xw = xbuf.bitcast(jnp.uint32)
    hw = hbuf.bitcast(jnp.uint32)
    fw = fbuf.bitcast(jnp.uint32)
    tb = (t0, t1, t2, t3)
    ub = (ur, ui)

    wcp.wait()
    _w_transform(wraw, wfreq, pbr, pbi, sr, si)
    wcp2 = pltpu.make_async_copy(w2_hbm, wraw, sems.at[4])
    wcp2.start()
    for b in range(B):
        xcps[2 * b].wait()
        xcps[2 * b + 1].wait()
        _conv_chunk(xw, b * P1, NB1, zbuf, wfreq, vr, vi, tb, ub, hw, 8 + b * P2)
        for c in range(2):
            n = 2 * P2 - T1
            hbuf[c, pl.ds(16 + b * 2 * P2 + T1, n), :] = jnp.zeros((n, H), bf)
    wcp2.wait()
    _w_transform(wraw, wfreq, pbr, pbi, sr, si)
    _conv_chunk(hw, 0, B * NB2, zbuf, wfreq, vr, vi, tb, ub, fw, 0)

    ntile = T2 // TT

    def ocopy(slot, b, t0_, sem_slot):
        return pltpu.make_async_copy(obuf.at[slot], o_hbm.at[b, pl.ds(t0_, TT)], osems.at[sem_slot])

    for b in range(B):
        ge = jnp.dot(g_ref[b], wg_ref[...], preferred_element_type=jnp.float32)

        def jbody(i, c, b=b, ge=ge):
            step = b * ntile + i
            slot = step & 1
            t0_ = pl.multiple_of(i * TT, 16)
            frow = pl.multiple_of(b * 2 * P3 + i * TT, 16)
            f = jnp.concatenate([fbuf[0, pl.ds(frow, TT), :], fbuf[1, pl.ds(frow, TT), :]], axis=1)
            fe = jnp.dot(f, wf_ref[...], preferred_element_type=jnp.float32)
            j = jnp.tanh(fe[:, None, :] + ge[None, :, :]).reshape(TT * U, D).astype(bf)
            o = jnp.dot(j, wo_ref[...], preferred_element_type=jnp.float32)

            @pl.when(step >= 2)
            def _():
                ocopy(slot, b, t0_, slot).wait()
            obuf[slot] = o.reshape(TT, U, D).astype(bf)
            ocopy(slot, b, t0_, slot).start()
            return c
        lax.fori_loop(0, ntile, jbody, 0)
    for slot in range(2):
        ocopy(slot, 0, 0, slot).wait()


def make(interpret=False, **kw):
    def fn(x, w1, w2, g, w_f, w_g, w_o):
        f32, bf = jnp.float32, jnp.bfloat16
        vm = lambda s, d: pltpu.VMEM(s, d)
        any_spec = pl.BlockSpec(memory_space=pl.ANY)
        vspec = pl.BlockSpec(memory_space=pltpu.VMEM)
        return pl.pallas_call(
            _kernel,
            in_specs=[any_spec, any_spec, any_spec, vspec, vspec, vspec, vspec],
            out_specs=any_spec,
            out_shape=jax.ShapeDtypeStruct((B, T2, U, D), bf),
            scratch_shapes=[
                vm((2, 2 * XR, H), bf), vm((2, 2 * HR, H), bf), vm((2, 2 * FR, H), bf),
                vm((K, D, D), bf), vm((N, 3, 2 * D, H), bf), vm((3, N, NB1, D), bf),
                vm((N, NB1, H), f32), vm((N, NB1, H), f32),
                vm((9, 8, 8, H), f32), vm((9, 8, 8, H), f32), vm((9, 8, 8, H), f32), vm((9, 8, 8, H), f32),
                vm((9, 8, 8, H), f32), vm((9, 8, 8, H), f32),
                vm((17, 16, H), f32), vm((17, 16, H), f32),
                vm((5, 4, 4, 16, H), f32), vm((5, 4, 4, 16, H), f32),
                vm((2, TT, U, D), bf),
                pltpu.SemaphoreType.DMA((5,)), pltpu.SemaphoreType.DMA((2,)),
            ],
            compiler_params=pltpu.CompilerParams(vmem_limit_bytes=120 * 1024 * 1024),
            interpret=interpret,
            name="rnnt_fft",
        )(x, w1, w2, g, w_f, w_g, w_o)
    return fn


_fn = make()


@jax.jit
def pallas_standalone__seq2seq_rnn_t_joint__speech_kernel(x, w1, w2, g, w_f, w_g, w_o):
    return _fn(x, w1, w2, g, w_f, w_g, w_o)
```

```python
import functools
import numpy as np
import jax
import jax.numpy as jnp
from jax import lax
import jax.experimental.pallas as pl
import jax.experimental.pallas.tpu as pltpu

B, T, D, K, U = 2, 16000, 256, 31, 8
H = D // 2
T1, T2 = T // 2, T // 4
N = 64
HOP = 46
MC = 32
NB1 = 176
NB2 = NB1 // 2
NC1 = B * NB1 // MC
NC2 = 6
NJOB = NC1 + NC2
P1 = NB1 * HOP
P2 = NB2 * HOP
P3 = NB2 * HOP // 2
XR = 8 + B * P1 + 24
HR = MC * NC2 * HOP + 64
FR = MC * NC2 * HOP // 2
XOFF, HOFF, FOFF = 0, XR, XR + HR
SEQR = XR + HR + FR
TT = 400
JSUB = 40
RS2 = float(np.sqrt(0.5))
HIMASK = np.uint32(0xFFFF0000)
OSCALE = 1.0 / (2 * N)
GC0 = float(np.sqrt(2.0 / np.pi))
GC1 = 0.044715
f32, bf16, u32 = jnp.float32, jnp.bfloat16, jnp.uint32


def fft8(xr, xi):
    a0r, a0i = xr[0] + xr[4], xi[0] + xi[4]
    a1r, a1i = xr[0] - xr[4], xi[0] - xi[4]
    a2r, a2i = xr[2] + xr[6], xi[2] + xi[6]
    a3r, a3i = xr[2] - xr[6], xi[2] - xi[6]
    a4r, a4i = xr[1] + xr[5], xi[1] + xi[5]
    a5r, a5i = xr[1] - xr[5], xi[1] - xi[5]
    a6r, a6i = xr[3] + xr[7], xi[3] + xi[7]
    a7r, a7i = xr[3] - xr[7], xi[3] - xi[7]
    e0r, e0i = a0r + a2r, a0i + a2i
    e2r, e2i = a0r - a2r, a0i - a2i
    e1r, e1i = a1r + a3i, a1i - a3r
    e3r, e3i = a1r - a3i, a1i + a3r
    o0r, o0i = a4r + a6r, a4i + a6i
    o2r, o2i = a4r - a6r, a4i - a6i
    o1r, o1i = a5r + a7i, a5i - a7r
    o3r, o3i = a5r - a7i, a5i + a7r
    t1r, t1i = (o1r + o1i) * RS2, (o1i - o1r) * RS2
    u, v = (o3i - o3r) * RS2, (o3r + o3i) * RS2
    yr = [e0r + o0r, e1r + t1r, e2r + o2i, e3r + u, e0r - o0r, e1r - t1r, e2r - o2i, e3r - u]
    yi = [e0i + o0i, e1i + t1i, e2i - o2r, e3i - v, e0i - o0i, e1i - t1i, e2i + o2r, e3i + v]
    return yr, yi


def ifft8(xr, xi):
    yi, yr = fft8(xi, xr)
    return yr, yi


def idft4(xr, xi):
    s02r, s02i = xr[0] + xr[2], xi[0] + xi[2]
    d02r, d02i = xr[0] - xr[2], xi[0] - xi[2]
    s13r, s13i = xr[1] + xr[3], xi[1] + xi[3]
    d13r, d13i = xr[1] - xr[3], xi[1] - xi[3]
    yr = [s02r + s13r, d02r - d13i, s02r - s13r, d02r + d13i]
    yi = [s02i + s13i, d02i + d13r, s02i - s13i, d02i - d13r]
    return yr, yi


def tw(ar, ai, num, den):
    num = num % den
    if num == 0:
        return ar, ai
    if num * 4 == den:
        return -ai, ar
    if num * 2 == den:
        return -ar, -ai
    if num * 4 == 3 * den:
        return ai, -ar
    if (num * 8) % den == 0:
        q = num * 8 // den
        if q == 1:
            return (ar - ai) * RS2, (ar + ai) * RS2
        if q == 3:
            return (ar + ai) * (-RS2), (ar - ai) * RS2
        if q == 5:
            return (ai - ar) * RS2, (ar + ai) * (-RS2)
        return (ar + ai) * RS2, (ai - ar) * RS2
    c = float(np.cos(2 * np.pi * num / den))
    s = float(np.sin(2 * np.pi * num / den))
    return ar * c - ai * s, ar * s + ai * c


def gelu_scaled(v):
    s = OSCALE
    t = v * v
    inner = v * (t * float(GC0 * GC1 * s * s * s) + float(GC0 * s))
    hv = v * float(0.5 * s)
    return hv + hv * jnp.tanh(inner)


def lo(w):
    return pltpu.bitcast(w << 16, f32)


def hi(w):
    return pltpu.bitcast(w & HIMASK, f32)


def pack2(a, b):
    return pltpu.pack_elementwise([a, b], packed_dtype=bf16)


class Gate:
    def __init__(self, zmask):
        self.z = zmask
        self.tok = None
        self.vtoks = []
        self.lv = 6

    def vpub(self, x):
        if self.lv > 0 and self.z is not None:
            self.vtoks.append(x)

    def mgate(self, w):
        if self.lv <= 0 or len(self.vtoks) < self.lv or self.vtoks[-self.lv] is None:
            return w
        x = self.vtoks[-self.lv]
        self.vtoks[-self.lv] = None
        tok = (x if x.dtype == u32 else pltpu.bitcast(x, u32)) & self.z
        head = w[0:8, :] | tok
        return jnp.concatenate([head, w[8:, :]], axis=0)

    def publish(self, g):
        self.tok = pltpu.bitcast(g[0:8, 0:H], u32) & self.z

    def gate_w(self, w):
        return w if self.tok is None else (w | self.tok)

    def gate_f(self, x):
        if self.tok is None:
            return x
        return pltpu.bitcast(pltpu.bitcast(x, u32) | self.tok, f32)


def chain(gens):
    for g in gens:
        yield from g


def interleave(mgen, mtot, vgen, vtot, lead):
    if mgen is None:
        for _ in vgen:
            pass
        return
    if vgen is None:
        for _ in mgen:
            pass
        return
    m_done = v_done = 0.0
    m_alive = v_alive = True
    while m_alive or v_alive:
        pick_v = v_alive and (not m_alive or (v_done - lead) / max(vtot - lead, 1.0) <= m_done / mtot)
        try:
            if pick_v:
                v_done += next(vgen)
            else:
                m_done += next(mgen)
        except StopIteration:
            if pick_v:
                v_alive = False
            else:
                m_alive = False


def g_fwd_pass1(src, tr, ti, gate):
    for n2 in range(8):
        xr, xi = [], []
        for n1 in range(8):
            w = src[pl.ds(8 * n1 + n2, 8, stride=2 * HOP), :]
            if n1 == 0:
                w = gate.gate_w(w)
            xr.append(lo(w))
            xi.append(hi(w))
        ar, ai = fft8(xr, xi)
        for k1 in range(8):
            br, bi = tw(ar[k1], ai[k1], -n2 * k1, N)
            tr[k1, n2] = br
            ti[k1, n2] = bi
        gate.vpub(br)
        yield 29


def g_fwd_pass2(tar, tai, tbr, tbi, zv, wrow0, gate):
    for k1 in range(8):
        la = [tar[k1, n] for n in range(8)]
        la[0] = gate.gate_f(la[0])
        ya_r, ya_i = fft8(la, [tai[k1, n] for n in range(8)])
        yb_r, yb_i = fft8([tbr[k1, n] for n in range(8)], [tbi[k1, n] for n in range(8)])
        for k2 in range(8):
            k = k1 + 8 * k2
            zv[0, k, pl.ds(wrow0, 8), :] = pack2(ya_r[k2] + ya_i[k2], yb_r[k2] + yb_i[k2])
            zv[1, k, pl.ds(wrow0, 8), :] = pack2(ya_r[k2], yb_r[k2])
            zv[2, k, pl.ds(wrow0, 8), :] = pack2(ya_i[k2], yb_i[k2])
        gate.vpub(yb_i[7])
        yield 38


def g_funit(seqw, src_row, col, zdst, wrow0, tb, z, gate):
    tar, tai, tbr, tbi = tb
    sub = seqw.at[col, pl.ds(src_row, 16 * HOP + 32), :]
    yield from g_fwd_pass1(sub, tar, tai, gate)
    yield from g_fwd_pass1(sub.at[pl.ds(HOP, 15 * HOP + 32), :], tbr, tbi, gate)
    views = [t.at[pl.ds(z, 8)] for t in tb]
    yield from g_fwd_pass2(*views, zdst.at[:, :, :, pl.ds(col * H, H)], wrow0, gate)


def g_mstep(k, zbuf, wf, vr, vi, gate):
    kn = (N - k) & (N - 1)

    def dot(a, b, wi):
        l = pltpu.bitcast(jnp.concatenate([gate.mgate(a[:, 0:H]), a[:, H:D], b], axis=1), bf16)
        g = jnp.dot(l, pltpu.bitcast(wf[k, wi], bf16), preferred_element_type=f32)
        gate.publish(g)
        return g
    g1 = dot(zbuf[0, k], zbuf[0, kn], 0)
    yield MC
    g2 = dot(zbuf[2, k], zbuf[1, kn], 1)
    vr[k] = g1 - g2
    yield MC
    g3 = dot(zbuf[1, k], zbuf[2, kn], 2)
    vi[k] = g1 - g3
    yield MC


def g_iunit(vr, vi, row0, ub, z, seqw, dst_row, gate):
    ur, ui = ub
    for k1 in range(8):
        xr = [vr[k1 + 8 * k2, pl.ds(row0, 8), :] for k2 in range(8)]
        xi = [vi[k1 + 8 * k2, pl.ds(row0, 8), :] for k2 in range(8)]
        xr[0] = gate.gate_f(xr[0])
        ar, ai = ifft8(xr, xi)
        for m2 in range(8):
            br, bi = tw(ar[m2], ai[m2], m2 * k1, N)
            ur[m2, k1] = br
            ui[m2, k1] = bi
        gate.vpub(br)
        yield 25
    urz, uiz = ur.at[pl.ds(z, 8)], ui.at[pl.ds(z, 8)]
    n = 8 * HOP // 2
    dst = [seqw.at[c, pl.ds(dst_row, n), :] for c in range(2)]
    for q in range(4):
        ys = []
        for m2 in (2 * q, 2 * q + 1):
            la = [urz[m2, k1] for k1 in range(8)]
            if m2 == 2 * q:
                la[0] = gate.gate_f(la[0])
            ys.append(ifft8(la, [uiz[m2, k1] for k1 in range(8)]))
        for m1 in range(6):
            m = 8 * m1 + 2 * q
            if m >= HOP:
                continue
            for part in range(2):
                va, vb = ys[0][part][m1], ys[1][part][m1]
                if m1 == 3:
                    va, vb = gate.gate_f(va), gate.gate_f(vb)
                a = gelu_scaled(va)
                b = gelu_scaled(vb)
                dst[part][pl.ds(m // 2, 8, stride=HOP // 2), :] = pack2(a, b)
            if m1 == 2:
                gate.vpub(b)
                yield 44
        gate.vpub(b)
        yield 31


def g_wslab(ww, slab, wf, pb, sb, z, gate):
    rows = pl.ds(pl.multiple_of(slab * 8, 8), 8)
    cat = lambda w: jnp.concatenate([lo(w), hi(w)], axis=0)
    for j in range(16):
        w0 = ww[0, 2 * j, rows, :]
        if j % 4 == 0:
            w0 = gate.gate_w(w0)
        vo0, vo1 = cat(w0), cat(ww[1, 2 * j, rows, :])
        if j == 0:
            pb[0, j], pb[1, j], pb[2, j], pb[3, j] = vo1, -vo0, -vo1, vo0
        else:
            ve0, ve1 = cat(ww[0, 2 * j - 1, rows, :]), cat(ww[1, 2 * j - 1, rows, :])
            pb[0, j], pb[1, j], pb[2, j], pb[3, j] = ve0 + vo1, ve1 - vo0, ve0 - vo1, ve1 + vo0
        if j % 4 == 3:
            gate.vpub(vo1[0:8])
            yield 34
    pbz = pb.at[pl.ds(z, 4)]
    sbz = sb.at[pl.ds(z, 2)]
    for which in range(2):
        for r in range(4):
            for j2 in range(4):
                xr, xi = [], []
                for j1 in range(4):
                    j = 4 * j1 + j2
                    pr_ = pbz[2 * which, j]
                    if j1 == 0:
                        pr_ = jnp.concatenate([gate.gate_f(pr_[0:8]), pr_[8:16]], axis=0)
                    a, b = tw(pr_, pbz[2 * which + 1, j], j * r, N)
                    xr.append(a)
                    xi.append(b)
                yr, yi = idft4(xr, xi)
                for k1 in range(4):
                    a, b = tw(yr[k1], yi[k1], j2 * k1, 16)
                    sb[0, r * 16 + k1 * 4 + j2] = a
                    sb[1, r * 16 + k1 * 4 + j2] = b
                gate.vpub(b[0:8])
                yield 26
        orow = pl.ds(pl.multiple_of(slab * 8 + which * H, 8), 8)
        for r in range(4):
            for k1 in range(4):
                lr_ = [sbz[0, r * 16 + k1 * 4 + j2] for j2 in range(4)]
                lr_[0] = jnp.concatenate([gate.gate_f(lr_[0][0:8]), lr_[0][8:16]], axis=0)
                yr, yi = idft4(lr_, [sbz[1, r * 16 + k1 * 4 + j2] for j2 in range(4)])
                for k2 in range(4):
                    k = 4 * (k1 + 4 * k2) + r
                    if which:
                        ms = (yi[k2], yi[k2] - yr[k2], yi[k2] + yr[k2])
                    else:
                        ms = (yr[k2], yr[k2] + yi[k2], yr[k2] - yi[k2])
                    for t, mm in enumerate(ms):
                        wf[k, t, orow, :] = pack2(mm[0:8], mm[8:16])
                gate.vpub(mm[0:8])
                yield 17


def _kernel(x_hbm, w1_hbm, w2_hbm, g_ref, wf_ref, wg_ref, wo_ref, o_hbm,
            seq, wraw1, wraw2, wfr1, wfr2, zA, zB, vAr, vAi, vBr, vBi,
            t0, t1, t2, t3, ur, ui, pb, sb, zz, obuf, sems, osems):
    def xcopy(b, c):
        return pltpu.make_async_copy(
            x_hbm.at[b, :, pl.ds(c * H, H)],
            seq.at[c, pl.ds(2 * XOFF + 16 + b * 2 * P1, T), :], sems.at[b * 2 + c])
    wcp1 = [pltpu.make_async_copy(w1_hbm.at[:, :, pl.ds(c * H, H)], wraw1.at[c], sems.at[4 + c]) for c in range(2)]
    wcp2 = [pltpu.make_async_copy(w2_hbm.at[:, :, pl.ds(c * H, H)], wraw2.at[c], sems.at[6 + c]) for c in range(2)]
    for cp in wcp1:
        cp.start()
    zero16 = lambda n: jnp.zeros((n, H), bf16)
    for c in range(2):
        seq[c, pl.ds(2 * XOFF, 16), :] = zero16(16)
        for b in range(B):
            n = 2 * P1 - T + (48 if b == B - 1 else 0)
            seq[c, pl.ds(2 * XOFF + 16 + b * 2 * P1 + T, n), :] = zero16(n)
        seq[c, pl.ds(2 * HOFF, 16), :] = zero16(16)
        n = 2 * HR - 16 - B * 2 * P2
        seq[c, pl.ds(2 * HOFF + 16 + B * 2 * P2, n), :] = zero16(n)
    zz[...] = jnp.zeros((8, H), u32)
    vBr[...] = jnp.zeros(vBr.shape, f32)
    vBi[...] = jnp.zeros(vBi.shape, f32)
    seqw = seq.bitcast(u32)
    tb, ub = (t0, t1, t2, t3), (ur, ui)
    nogate = Gate(None)

    for cp in wcp1:
        cp.wait()
    for c in range(2):
        xcopy(0, c).start()
    for cp in wcp2:
        cp.start()
    ww1 = wraw1.bitcast(u32)
    ww2 = wraw2.bitcast(u32)

    def w1body(s, c):
        for _ in g_wslab(ww1, s, wfr1, pb, sb, s >> 16, nogate):
            pass
        return c
    with jax.named_scope('ph_W1'):
        lax.fori_loop(0, D // 16, w1body, 0)
    for c in range(2):
        xcopy(0, c).wait()
    for c in range(2):
        xcopy(1, c).start()
    for cp in wcp2:
        cp.wait()

    def src_row(job, g16):
        base = jnp.where(job < NC1, XOFF + job * (MC * HOP), HOFF + (job - NC1) * (MC * HOP))
        return pl.multiple_of(base + g16 * (16 * HOP), 8)

    def dst_row(job, g8):
        base = jnp.where(job < NC1, HOFF + 8 + job * (MC * HOP // 2), FOFF + (job - NC1) * (MC * HOP // 2))
        return pl.multiple_of(base + g8 * (8 * HOP // 2), 8)

    def f0body(g16, c):
        for col in range(2):
            for _ in g_funit(seqw, src_row(0, g16), col, zA, pl.multiple_of(g16 * 8, 8), tb, g16 >> 16, nogate):
                pass
        return c
    with jax.named_scope('ph_F0'):
        lax.fori_loop(0, MC // 16, f0body, 0)

    LEAD = 150.0

    def half_step(s, h, par, with_w):
        zM, zF = (zA, zB) if par == 0 else (zB, zA)
        vM, vI = ((vAr, vAi), (vBr, vBi)) if par == 0 else ((vBr, vBi), (vAr, vAi))
        wfr = wfr1
        z = h >> 16
        gate = Gate(zz[...])
        jf = jnp.minimum(s + 1, NJOB - 1)
        ji = jnp.maximum(s - 1, 0)
        vg = []
        for col in range(2):
            vg.append(g_funit(seqw, src_row(jf, h), col, zF, pl.multiple_of(h * 8, 8), tb, z, gate))
            vg.append(g_iunit(vI[0], vI[1], pl.multiple_of(h * 16 + col * 8, 8), ub, z, seqw,
                              dst_row(ji, 2 * h + col), gate))
        vtot = 2 * (16 * 29 + 8 * 38) + 2 * (8 * 25 + 4 * 75)
        if with_w:
            vg.append(g_wslab(ww2, 2 * s + h, wfr2, pb, sb, z, gate))
            vtot += 4 * 34 + 2 * (16 * 26 + 16 * 17)
        return zM, vM, gate, vg, vtot

    def run_half(s, h, par, with_w, wsel):
        zM, vM, gate, vg, vtot = half_step(s, h, par, with_w)
        wfr = wfr1 if wsel == 1 else wfr2
        mg = [g_mstep(h * 32 + a, zM, wfr, vM[0], vM[1], gate) for a in range(32)]
        interleave(chain(mg), 32 * 3 * MC, chain(vg), vtot, LEAD)

    def step(s, par, with_w, wsel):
        def hb(h, c):
            run_half(s, h, par, with_w, wsel)
            return c
        lax.fori_loop(0, 2, hb, 0)

    def pair_loop(p0, p1, with_w, wsel):
        def pb_(p, c):
            step(2 * p, 0, with_w, wsel)
            step(2 * p + 1, 1, with_w, wsel)
            return c
        lax.fori_loop(p0, p1, pb_, 0)

    with jax.named_scope('ph_c1w'):
        pair_loop(0, 2, True, 1)
        for c in range(2):
            xcopy(1, c).wait()
        pair_loop(2, 4, True, 1)
    with jax.named_scope('ph_c1'):
        pair_loop(4, 5, False, 1)
        step(jnp.int32(10), 0, False, 1)
    with jax.named_scope('ph_c2a'):
        step(jnp.int32(11), 1, False, 2)
    for c in range(2):
        for b in range(B):
            n = 2 * P2 - T1
            seq[c, pl.ds(2 * HOFF + 16 + b * 2 * P2 + T1, n), :] = zero16(n)
    with jax.named_scope('ph_c2b'):
        pair_loop(6, 8, False, 2)
        step(jnp.int32(16), 0, False, 2)

    def ilast(g8, c):
        for _ in g_iunit(vAr, vAi, pl.multiple_of(g8 * 8, 8), ub, g8 >> 16, seqw, dst_row(NJOB - 1, g8), nogate):
            pass
        return c
    lax.fori_loop(0, 2, ilast, 0)

    ntile = T2 // TT

    def ocopy(slot, b, t0_):
        return pltpu.make_async_copy(obuf.at[slot], o_hbm.at[b, pl.ds(t0_, TT)], osems.at[slot])

    for b in range(B):
        ge = jnp.dot(g_ref[b], wg_ref[...], preferred_element_type=f32)

        def jbody(i, c, b=b, ge=ge):
            step_ = b * ntile + i
            slot = step_ & 1
            t0_ = pl.multiple_of(i * TT, 16)

            @pl.when(step_ >= 2)
            def _():
                ocopy(slot, b, t0_).wait()
            frow = pl.multiple_of(2 * FOFF + b * 2 * P3 + i * TT, 16)
            f = jnp.concatenate([seq[0, pl.ds(frow, TT), :], seq[1, pl.ds(frow, TT), :]], axis=1)
            fe = jnp.dot(f, wf_ref[...], preferred_element_type=f32)
            for s_ in range(TT // JSUB):
                fes = fe[s_ * JSUB:(s_ + 1) * JSUB]
                j = jnp.tanh(fes[:, None, :] + ge[None, :, :]).reshape(JSUB * U, D).astype(bf16)
                o = jnp.dot(j, wo_ref[...], preferred_element_type=f32)
                obuf[slot, pl.ds(s_ * JSUB, JSUB)] = o.reshape(JSUB, U, D).astype(bf16)
            ocopy(slot, b, t0_).start()
            return c
        with jax.named_scope('ph_J'):
            lax.fori_loop(0, ntile, jbody, 0)
    for slot in range(2):
        ocopy(slot, 0, 0).wait()


def make(interpret=False):
    def fn(x, w1, w2, g, w_f, w_g, w_o):
        vm = pltpu.VMEM
        any_spec = pl.BlockSpec(memory_space=pl.ANY)
        vspec = pl.BlockSpec(memory_space=pltpu.VMEM)
        zsh = (3, N, MC // 2, D)
        vsh = (N, MC, H)
        return pl.pallas_call(
            _kernel,
            in_specs=[any_spec, any_spec, any_spec, vspec, vspec, vspec, vspec],
            out_specs=any_spec,
            out_shape=jax.ShapeDtypeStruct((B, T2, U, D), bf16),
            scratch_shapes=[
                vm((2, 2 * SEQR, H), bf16), vm((2, K, D, H), bf16), vm((2, K, D, H), bf16),
                vm((N, 3, D, H), u32), vm((N, 3, D, H), u32), vm(zsh, u32), vm(zsh, u32),
                vm(vsh, f32), vm(vsh, f32), vm(vsh, f32), vm(vsh, f32),
                vm((9, 8, 8, H), f32), vm((9, 8, 8, H), f32), vm((9, 8, 8, H), f32), vm((9, 8, 8, H), f32),
                vm((9, 8, 8, H), f32), vm((9, 8, 8, H), f32),
                vm((5, 16, 16, H), f32), vm((3, 64, 16, H), f32), vm((8, H), u32),
                vm((2, TT, U, D), bf16),
                pltpu.SemaphoreType.DMA((8,)), pltpu.SemaphoreType.DMA((2,)),
            ],
            compiler_params=pltpu.CompilerParams(vmem_limit_bytes=124 * 1024 * 1024),
            interpret=interpret,
            name="rnnt_fft2",
        )(x, w1, w2, g, w_f, w_g, w_o)
    return fn


_fn = make()


@jax.jit
def pallas_standalone__seq2seq_rnn_t_joint__speech_kernel(x, w1, w2, g, w_f, w_g, w_o):
    return _fn(x, w1, w2, g, w_f, w_g, w_o)
```

```python
import functools
import numpy as np
import jax
import jax.numpy as jnp
from jax import lax
import jax.experimental.pallas as pl
import jax.experimental.pallas.tpu as pltpu

B, T, D, K, U = 2, 16000, 256, 31, 8
H = D // 2
T1, T2 = T // 2, T // 4
N = 64
HOP = 46
MC = 32
NB1 = 176
NB2 = NB1 // 2
NC1 = B * NB1 // MC
NC2 = 6
NJOB = NC1 + NC2
P1 = NB1 * HOP
P2 = NB2 * HOP
P3 = NB2 * HOP // 2
XR = 8 + B * P1 + 24
HR = MC * NC2 * HOP + 64
FR = MC * NC2 * HOP // 2
XOFF, HOFF, FOFF = 0, XR, XR + HR
SEQR = XR + HR + FR
FINE = 1
TT = 400
JSUB = 40
RS2 = float(np.sqrt(0.5))
HIMASK = np.uint32(0xFFFF0000)
OSCALE = 1.0 / (2 * N)
HS1 = 0.5 * OSCALE
S2 = OSCALE * HS1
HS2 = 0.5 * S2
GC0 = float(np.sqrt(2.0 / np.pi))
GC1 = 0.044715
f32, bf16, u32 = jnp.float32, jnp.bfloat16, jnp.uint32


def fft8(xr, xi):
    a0r, a0i = xr[0] + xr[4], xi[0] + xi[4]
    a1r, a1i = xr[0] - xr[4], xi[0] - xi[4]
    a2r, a2i = xr[2] + xr[6], xi[2] + xi[6]
    a3r, a3i = xr[2] - xr[6], xi[2] - xi[6]
    a4r, a4i = xr[1] + xr[5], xi[1] + xi[5]
    a5r, a5i = xr[1] - xr[5], xi[1] - xi[5]
    a6r, a6i = xr[3] + xr[7], xi[3] + xi[7]
    a7r, a7i = xr[3] - xr[7], xi[3] - xi[7]
    e0r, e0i = a0r + a2r, a0i + a2i
    e2r, e2i = a0r - a2r, a0i - a2i
    e1r, e1i = a1r + a3i, a1i - a3r
    e3r, e3i = a1r - a3i, a1i + a3r
    o0r, o0i = a4r + a6r, a4i + a6i
    o2r, o2i = a4r - a6r, a4i - a6i
    o1r, o1i = a5r + a7i, a5i - a7r
    o3r, o3i = a5r - a7i, a5i + a7r
    t1r, t1i = (o1r + o1i) * RS2, (o1i - o1r) * RS2
    u, v = (o3i - o3r) * RS2, (o3r + o3i) * RS2
    yr = [e0r + o0r, e1r + t1r, e2r + o2i, e3r + u, e0r - o0r, e1r - t1r, e2r - o2i, e3r - u]
    yi = [e0i + o0i, e1i + t1i, e2i - o2r, e3i - v, e0i - o0i, e1i - t1i, e2i + o2r, e3i + v]
    return yr, yi


def ifft8(xr, xi):
    yi, yr = fft8(xi, xr)
    return yr, yi


def idft4(xr, xi):
    s02r, s02i = xr[0] + xr[2], xi[0] + xi[2]
    d02r, d02i = xr[0] - xr[2], xi[0] - xi[2]
    s13r, s13i = xr[1] + xr[3], xi[1] + xi[3]
    d13r, d13i = xr[1] - xr[3], xi[1] - xi[3]
    yr = [s02r + s13r, d02r - d13i, s02r - s13r, d02r + d13i]
    yi = [s02i + s13i, d02i + d13r, s02i - s13i, d02i - d13r]
    return yr, yi


def tw(ar, ai, num, den):
    num = num % den
    if num == 0:
        return ar, ai
    if num * 4 == den:
        return -ai, ar
    if num * 2 == den:
        return -ar, -ai
    if num * 4 == 3 * den:
        return ai, -ar
    if (num * 8) % den == 0:
        q = num * 8 // den
        if q == 1:
            return (ar - ai) * RS2, (ar + ai) * RS2
        if q == 3:
            return (ar + ai) * (-RS2), (ar - ai) * RS2
        if q == 5:
            return (ai - ar) * RS2, (ar + ai) * (-RS2)
        return (ar + ai) * RS2, (ai - ar) * RS2
    c = float(np.cos(2 * np.pi * num / den))
    s = float(np.sin(2 * np.pi * num / den))
    return ar * c - ai * s, ar * s + ai * c


def gelu_consts(s):
    return float(GC0 * GC1 * s * s * s), float(GC0 * s)


def gelu_scaled(v, c3, c1):
    inner = v * ((v * v) * c3 + c1)
    return v * (jnp.tanh(inner) + 1.0)


def lo(w):
    return pltpu.bitcast(w << 16, f32)


def hi(w):
    return pltpu.bitcast(w & HIMASK, f32)


def pack2(a, b):
    return pltpu.pack_elementwise([a, b], packed_dtype=bf16)


class Gate:
    def __init__(self, zmask, lm=None, lv=None, every=None):
        self.z = zmask
        self.tok = None
        self.mtoks = []
        self.lm = 2 if lm is None else lm
        self.every = 1 if every is None else every
        self.cnt = 0
        self.vtoks = []
        self.lv = 8 if lv is None else lv

    def vpub(self, x):
        if self.lv > 0 and self.z is not None:
            self.vtoks.append(x)

    def mgate(self, w):
        if self.lv <= 0 or len(self.vtoks) < self.lv or self.vtoks[-self.lv] is None:
            return w
        x = self.vtoks[-self.lv]
        self.vtoks[-self.lv] = None
        tok = (x if x.dtype == u32 else pltpu.bitcast(x, u32)) & self.z
        head = w[0:8, :] | tok
        return jnp.concatenate([head, w[8:, :]], axis=0)

    def publish(self, g):
        if self.z is not None:
            self.mtoks.append(g[0:8, 0:H])

    def _tok(self):
        if self.z is None or len(self.mtoks) < self.lm:
            return None
        self.cnt += 1
        if self.cnt % self.every != 0:
            return None
        t = self.mtoks[-self.lm]
        if t.dtype != u32:
            t = pltpu.bitcast(t, u32) & self.z
            self.mtoks[-self.lm] = t
        return t

    def gate_w(self, w):
        t = self._tok()
        return w if t is None else (w | t)

    def gate_f(self, x):
        t = self._tok()
        if t is None:
            return x
        return pltpu.bitcast(pltpu.bitcast(x, u32) | t, f32)


def chain(gens):
    for g in gens:
        yield from g


def interleave(mgen, mtot, vgen, vtot, lead):
    if mgen is None:
        for _ in vgen:
            pass
        return
    if vgen is None:
        for _ in mgen:
            pass
        return
    m_done = v_done = 0.0
    m_alive = v_alive = True
    while m_alive or v_alive:
        pick_v = v_alive and (not m_alive or (v_done - lead) / max(vtot - lead, 1.0) <= m_done / mtot)
        try:
            if pick_v:
                v_done += next(vgen)
            else:
                m_done += next(mgen)
        except StopIteration:
            if pick_v:
                v_alive = False
            else:
                m_alive = False


def g_fwd_pass1(src, tr, ti, gate):
    for n2 in range(8):
        xr, xi = [], []
        for n1 in range(8):
            w = src[pl.ds(8 * n1 + n2, 8, stride=2 * HOP), :]
            if n1 == 0:
                w = gate.gate_w(w)
            xr.append(lo(w))
            xi.append(hi(w))
        ar, ai = fft8(xr, xi)
        if FINE:
            gate.vpub(ar[7])
            yield 19
            ar[1] = gate.gate_f(ar[1])
        for k1 in range(8):
            br, bi = tw(ar[k1], ai[k1], -n2 * k1, N)
            tr[k1, n2] = br
            ti[k1, n2] = bi
        gate.vpub(br)
        yield (10 if FINE else 29)


def g_fwd_pass2(tar, tai, tbr, tbi, zv, wrow0, gate):
    for k1 in range(8):
        la = [tar[k1, n] for n in range(8)]
        la[0] = gate.gate_f(la[0])
        ya_r, ya_i = fft8(la, [tai[k1, n] for n in range(8)])
        if FINE:
            gate.vpub(ya_i[7])
            yield 14
        lb = [tbr[k1, n] for n in range(8)]
        if FINE:
            lb[0] = gate.gate_f(lb[0])
        yb_r, yb_i = fft8(lb, [tbi[k1, n] for n in range(8)])
        for k2 in range(8):
            if FINE and k2 == 4:
                gate.vpub(yb_i[3])
                yield 14
                ya_r[4] = gate.gate_f(ya_r[4])
            k = k1 + 8 * k2
            zv[0, k, pl.ds(wrow0, 8), :] = pack2(ya_r[k2] + ya_i[k2], yb_r[k2] + yb_i[k2])
            zv[1, k, pl.ds(wrow0, 8), :] = pack2(ya_r[k2], yb_r[k2])
            zv[2, k, pl.ds(wrow0, 8), :] = pack2(ya_i[k2], yb_i[k2])
        gate.vpub(yb_i[7])
        yield (10 if FINE else 38)


def g_funit(seqw, src_row, col, zdst, wrow0, tb, z, gate):
    tar, tai, tbr, tbi = tb
    sub = seqw.at[col, pl.ds(src_row, 16 * HOP + 32), :]
    yield from g_fwd_pass1(sub, tar, tai, gate)
    yield from g_fwd_pass1(sub.at[pl.ds(HOP, 15 * HOP + 32), :], tbr, tbi, gate)
    views = [t.at[pl.ds(z, 8)] for t in tb]
    yield from g_fwd_pass2(*views, zdst.at[:, :, :, pl.ds(col * H, H)], wrow0, gate)


def g_mstep(k, zbuf, wf, vr, vi, gate):
    kn = (N - k) & (N - 1)

    def dot(a, b, wi):
        l = pltpu.bitcast(jnp.concatenate([gate.mgate(a[:, 0:H]), a[:, H:D], b], axis=1), bf16)
        g = jnp.dot(l, pltpu.bitcast(wf[k, wi], bf16), preferred_element_type=f32)
        gate.publish(g)
        return g
    g1 = dot(zbuf[0, k], zbuf[0, kn], 0)
    yield MC
    g2 = dot(zbuf[2, k], zbuf[1, kn], 1)
    vr[k] = g1 - g2
    yield MC
    g3 = dot(zbuf[1, k], zbuf[2, kn], 2)
    vi[k] = g1 - g3
    yield MC


def g_iunit(vr, vi, row0, ub, z, seqw, dst_row, gate, gc):
    ur, ui = ub
    for k1 in range(8):
        xr = [vr[k1 + 8 * k2, pl.ds(row0, 8), :] for k2 in range(8)]
        xi = [vi[k1 + 8 * k2, pl.ds(row0, 8), :] for k2 in range(8)]
        xr[0] = gate.gate_f(xr[0])
        ar, ai = ifft8(xr, xi)
        if FINE:
            gate.vpub(ar[7])
            yield 15
            ar[1] = gate.gate_f(ar[1])
        for m2 in range(8):
            br, bi = tw(ar[m2], ai[m2], m2 * k1, N)
            ur[m2, k1] = br
            ui[m2, k1] = bi
        gate.vpub(br)
        yield (10 if FINE else 25)
    urz, uiz = ur.at[pl.ds(z, 8)], ui.at[pl.ds(z, 8)]
    n = 8 * HOP // 2
    dst = [seqw.at[c, pl.ds(dst_row, n), :] for c in range(2)]
    for q in range(4):
        ys = []
        for m2 in (2 * q, 2 * q + 1):
            la = [urz[m2, k1] for k1 in range(8)]
            if m2 == 2 * q:
                la[0] = gate.gate_f(la[0])
            ys.append(ifft8(la, [uiz[m2, k1] for k1 in range(8)]))
        for m1 in range(6):
            m = 8 * m1 + 2 * q
            if m >= HOP:
                continue
            for part in range(2):
                va, vb = ys[0][part][m1], ys[1][part][m1]
                if m1 == 3 or (FINE and m1 in (1, 5) and part == 0):
                    va, vb = gate.gate_f(va), gate.gate_f(vb)
                a = gelu_scaled(va, *gc)
                b = gelu_scaled(vb, *gc)
                dst[part][pl.ds(m // 2, 8, stride=HOP // 2), :] = pack2(a, b)
            if FINE and m1 == 0:
                gate.vpub(b)
                yield 30
            if m1 == 2:
                gate.vpub(b)
                yield (14 if FINE else 44)
            if FINE and m1 == 4:
                gate.vpub(b)
                yield 17
        gate.vpub(b)
        yield (14 if FINE else 31)


def g_wslab(ww, slab, wf, pb, sb, z, gate):
    rows = pl.ds(pl.multiple_of(slab * 8, 8), 8)
    for j2 in range(4):
        raw = []
        for j1 in range(4):
            j = 4 * j1 + j2
            w0 = ww[0, 2 * j, rows, :]
            if j1 == 0:
                w0 = gate.gate_w(w0)
            w1_ = ww[1, 2 * j, rows, :]
            we = (ww[0, 2 * j - 1, rows, :], ww[1, 2 * j - 1, rows, :]) if j > 0 else None
            raw.append((w0, w1_, we))
        for ab, un in enumerate((lo, hi)):
            pq = []
            for (w0, w1_, we) in raw:
                vo0, vo1 = un(w0), un(w1_)
                if we is None:
                    pq.append(((vo1, -vo0), (-vo1, vo0)))
                else:
                    ve0, ve1 = un(we[0]), un(we[1])
                    pq.append(((ve0 + vo1, ve1 - vo0), (ve0 - vo1, ve1 + vo0)))
            for which in range(2):
                for r in range(4):
                    xr, xi = [], []
                    for j1 in range(4):
                        pr_, pi_ = pq[j1][which]
                        if j1 == 0 and (r > 0 or which > 0 or ab > 0):
                            pr_ = gate.gate_f(pr_)
                        a, b = tw(pr_, pi_, (4 * j1 + j2) * r, N)
                        xr.append(a)
                        xi.append(b)
                    yr, yi = idft4(xr, xi)
                    for k1 in range(4):
                        a, b = tw(yr[k1], yi[k1], j2 * k1, 16)
                        sb[which, 0, r * 16 + k1 * 4 + j2, ab] = a
                        sb[which, 1, r * 16 + k1 * 4 + j2, ab] = b
                    gate.vpub(b)
                    yield 12
    sbz = sb.at[pl.ds(z, 2)]
    for which in range(2):
        orow = pl.ds(pl.multiple_of(slab * 8 + which * H, 8), 8)
        for r in range(4):
            for k1 in range(4):
                res = []
                for ab in range(2):
                    lr_ = [sbz[which, 0, r * 16 + k1 * 4 + j2, ab] for j2 in range(4)]
                    if ab == 0:
                        lr_[0] = gate.gate_f(lr_[0])
                    yr, yi = idft4(lr_, [sbz[which, 1, r * 16 + k1 * 4 + j2, ab] for j2 in range(4)])
                    if which:
                        res.append([(yi[k2], yi[k2] - yr[k2], yi[k2] + yr[k2]) for k2 in range(4)])
                    else:
                        res.append([(yr[k2], yr[k2] + yi[k2], yr[k2] - yi[k2]) for k2 in range(4)])
                for k2 in range(4):
                    k = 4 * (k1 + 4 * k2) + r
                    for t in range(3):
                        wf[k, t, orow, :] = pack2(res[0][k2][t], res[1][k2][t])
                gate.vpub(res[1][3][2])
                yield 16


def _kernel(x_hbm, w1_hbm, w2_hbm, g_ref, wf_ref, wg_ref, wo_ref, o_hbm,
            seq, wraw1, wraw2, wfr1, wfr2, zA, zB, vAr, vAi, vBr, vBi,
            t0, t1, t2, t3, ur, ui, pb, sb, zz, obuf, sems, osems, w1sems, xsems):
    XQ = T // 4

    def xcopy(b, q, c):
        r0, n = (0, T) if q is None else (q * XQ, XQ)
        return pltpu.make_async_copy(
            x_hbm.at[b, pl.ds(r0, n), pl.ds(c * H, H)],
            seq.at[c, pl.ds(2 * XOFF + 16 + b * 2 * P1 + r0, n), :],
            xsems.at[(8 if q is None else 2 * q) + c])

    def xstart(b, q):
        for c in range(2):
            xcopy(b, q, c).start()

    def xwait(b, q):
        for c in range(2):
            xcopy(b, q, c).wait()
    WG = 4

    def w1copy(grp, c):
        rows = pl.ds(grp * (D // WG), D // WG)
        return pltpu.make_async_copy(w1_hbm.at[:, rows, pl.ds(c * H, H)], wraw1.at[c, :, rows, :], w1sems.at[grp * 2 + c])
    wcp1 = [w1copy(grp, c) for grp in range(WG) for c in range(2)]
    wcp2 = [pltpu.make_async_copy(w2_hbm.at[:, :, pl.ds(c * H, H)], wraw2.at[c], sems.at[6 + c]) for c in range(2)]
    for cp in wcp1:
        cp.start()
    xstart(0, 0)
    zero16 = lambda n: jnp.zeros((n, H), bf16)
    for c in range(2):
        seq[c, pl.ds(2 * XOFF, 16), :] = zero16(16)
        for b in range(B):
            n = 2 * P1 - T + (48 if b == B - 1 else 0)
            seq[c, pl.ds(2 * XOFF + 16 + b * 2 * P1 + T, n), :] = zero16(n)
        seq[c, pl.ds(2 * HOFF, 16), :] = zero16(16)
        n = 2 * HR - 16 - B * 2 * P2
        seq[c, pl.ds(2 * HOFF + 16 + B * 2 * P2, n), :] = zero16(n)
    zz[...] = jnp.zeros((8, H), u32)
    vBr[...] = jnp.zeros(vBr.shape, f32)
    vBi[...] = jnp.zeros(vBi.shape, f32)
    seqw = seq.bitcast(u32)
    tb, ub = (t0, t1, t2, t3), (ur, ui)
    nogate = Gate(None)

    ww1 = wraw1.bitcast(u32)
    ww2 = wraw2.bitcast(u32)

    def w1body(s, c):
        for _ in g_wslab(ww1, s, wfr1, pb, sb, s >> 16, nogate):
            pass
        return c
    with jax.named_scope('ph_W1'):
        for grp in range(WG):
            for c in range(2):
                w1copy(grp, c).wait()
            if grp == 1:
                xstart(0, 1)
                xstart(0, 2)
            if grp == 2:
                for cp in wcp2:
                    cp.start()
            if grp == 3:
                xstart(0, 3)
            n = D // 16 // WG
            lax.fori_loop(grp * n, (grp + 1) * n, w1body, 0)
    with jax.named_scope('ph_xwait0'):
        xwait(0, 0)
    xstart(1, None)

    def src_row(job, g16):
        base = jnp.where(job < NC1, XOFF + job * (MC * HOP), HOFF + (job - NC1) * (MC * HOP))
        return pl.multiple_of(base + g16 * (16 * HOP), 8)

    def dst_row(job, g8):
        base = jnp.where(job < NC1, HOFF + 8 + job * (MC * HOP // 2), FOFF + (job - NC1) * (MC * HOP // 2))
        return pl.multiple_of(base + g8 * (8 * HOP // 2), 8)

    def f0body(g16, c):
        for col in range(2):
            for _ in g_funit(seqw, src_row(0, g16), col, zA, pl.multiple_of(g16 * 8, 8), tb, g16 >> 16, nogate):
                pass
        return c
    with jax.named_scope('ph_F0'):
        lax.fori_loop(0, MC // 16, f0body, 0)

    LEAD = 0.0

    def half_step(s, h, par, with_w):
        zM, zF = (zA, zB) if par == 0 else (zB, zA)
        vM, vI = ((vAr, vAi), (vBr, vBi)) if par == 0 else ((vBr, vBi), (vAr, vAi))
        wfr = wfr1
        z = h >> 16
        gate = Gate(zz[...])
        jf = jnp.minimum(s + 1, NJOB - 1)
        ji = jnp.maximum(s - 1, 0)
        ca, cb = gelu_consts(OSCALE), gelu_consts(S2)
        gc = (jnp.where(ji < NC1, ca[0], cb[0]).astype(f32), jnp.where(ji < NC1, ca[1], cb[1]).astype(f32))
        vg = []
        for col in range(2):
            vg.append(g_funit(seqw, src_row(jf, h), col, zF, pl.multiple_of(h * 8, 8), tb, z, gate))
            vg.append(g_iunit(vI[0], vI[1], pl.multiple_of(h * 16 + col * 8, 8), ub, z, seqw,
                              dst_row(ji, 2 * h + col), gate, gc))
        vtot = 2 * (16 * 29 + 8 * 38) + 2 * (8 * 25 + 4 * 75)
        if with_w:
            vg.append(g_wslab(ww2, 2 * s + h, wfr2, pb, sb, z, gate))
            vtot += 64 * 12 + 32 * 16
        return zM, vM, gate, vg, vtot

    def run_half(s, h, par, with_w, wsel):
        zM, vM, gate, vg, vtot = half_step(s, h, par, with_w)
        wfr = wfr1 if wsel == 1 else wfr2
        mg = [g_mstep(h * 32 + a, zM, wfr, vM[0], vM[1], gate) for a in range(32)]
        interleave(chain(mg), 32 * 3 * MC, chain(vg), vtot, LEAD)

    def step(s, par, with_w, wsel):
        def hb(h, c):
            run_half(s, h, par, with_w, wsel)
            return c
        lax.fori_loop(0, 2, hb, 0)

    def pair_loop(p0, p1, with_w, wsel):
        def pb_(p, c):
            if with_w:
                @pl.when(p == 1)
                def _():
                    xwait(0, 3)

                @pl.when(p == 2)
                def _():
                    xwait(1, None)
            step(2 * p, 0, with_w, wsel)
            step(2 * p + 1, 1, with_w, wsel)
            return c
        lax.fori_loop(p0, p1, pb_, 0)

    with jax.named_scope('ph_c1w'):
        xwait(0, 1)
        xwait(0, 2)
        for cp in wcp2:
            cp.wait()
        pair_loop(0, 4, True, 1)
    with jax.named_scope('ph_c1'):
        pair_loop(4, 5, False, 1)
        step(jnp.int32(10), 0, False, 1)
    with jax.named_scope('ph_c2a'):
        step(jnp.int32(11), 1, False, 2)
    for c in range(2):
        for b in range(B):
            n = 2 * P2 - T1
            seq[c, pl.ds(2 * HOFF + 16 + b * 2 * P2 + T1, n), :] = zero16(n)
    with jax.named_scope('ph_c2b'):
        pair_loop(6, 8, False, 2)
        step(jnp.int32(16), 0, False, 2)

    def ilast(g8, c):
        for _ in g_iunit(vAr, vAi, pl.multiple_of(g8 * 8, 8), ub, g8 >> 16, seqw, dst_row(NJOB - 1, g8), nogate, gelu_consts(S2)):
            pass
        return c
    with jax.named_scope('ph_ilast'):
        lax.fori_loop(0, 2, ilast, 0)

    ntile = T2 // TT

    def ocopy(slot, b, t0_):
        return pltpu.make_async_copy(obuf.at[slot], o_hbm.at[b, pl.ds(t0_, TT)], osems.at[slot])

    for b in range(B):
        ge = jnp.dot(g_ref[b], wg_ref[...], preferred_element_type=f32)

        def jbody(i, c, b=b, ge=ge):
            step_ = b * ntile + i
            slot = step_ & 1
            t0_ = pl.multiple_of(i * TT, 16)

            @pl.when(step_ >= 2)
            def _():
                ocopy(slot, b, t0_).wait()
            frow = pl.multiple_of(2 * FOFF + b * 2 * P3 + i * TT, 16)
            f = jnp.concatenate([seq[0, pl.ds(frow, TT), :], seq[1, pl.ds(frow, TT), :]], axis=1)
            fe = jnp.dot(f, wf_ref[...], preferred_element_type=f32) * HS2
            for s_ in range(TT // JSUB):
                fes = fe[s_ * JSUB:(s_ + 1) * JSUB]
                j = jnp.tanh(fes[:, None, :] + ge[None, :, :]).reshape(JSUB * U, D).astype(bf16)
                o = jnp.dot(j, wo_ref[...], preferred_element_type=f32)
                obuf[slot, pl.ds(s_ * JSUB, JSUB)] = o.reshape(JSUB, U, D).astype(bf16)
            ocopy(slot, b, t0_).start()
            return c
        with jax.named_scope('ph_J'):
            lax.fori_loop(0, ntile, jbody, 0)
    with jax.named_scope('ph_tail'):
        for slot in range(2):
            ocopy(slot, 0, 0).wait()


def make(interpret=False):
    def fn(x, w1, w2, g, w_f, w_g, w_o):
        vm = pltpu.VMEM
        any_spec = pl.BlockSpec(memory_space=pl.ANY)
        vspec = pl.BlockSpec(memory_space=pltpu.VMEM)
        zsh = (3, N, MC // 2, D)
        vsh = (N, MC, H)
        return pl.pallas_call(
            _kernel,
            in_specs=[any_spec, any_spec, any_spec, vspec, vspec, vspec, vspec],
            out_specs=any_spec,
            out_shape=jax.ShapeDtypeStruct((B, T2, U, D), bf16),
            scratch_shapes=[
                vm((2, 2 * SEQR, H), bf16), vm((2, K, D, H), bf16), vm((2, K, D, H), bf16),
                vm((N, 3, D, H), u32), vm((N, 3, D, H), u32), vm(zsh, u32), vm(zsh, u32),
                vm(vsh, f32), vm(vsh, f32), vm(vsh, f32), vm(vsh, f32),
                vm((9, 8, 8, H), f32), vm((9, 8, 8, H), f32), vm((9, 8, 8, H), f32), vm((9, 8, 8, H), f32),
                vm((9, 8, 8, H), f32), vm((9, 8, 8, H), f32),
                vm((8, H), f32), vm((3, 2, 64, 2, 8, H), f32), vm((8, H), u32),
                vm((2, TT, U, D), bf16),
                pltpu.SemaphoreType.DMA((8,)), pltpu.SemaphoreType.DMA((2,)), pltpu.SemaphoreType.DMA((8,)),
                pltpu.SemaphoreType.DMA((10,)),
            ],
            compiler_params=pltpu.CompilerParams(vmem_limit_bytes=124 * 1024 * 1024),
            interpret=interpret,
            name="rnnt_fft2",
        )(x, w1, w2, g, w_f, w_g, w_o)
    return fn


_fn = make()


@jax.jit
def pallas_standalone__seq2seq_rnn_t_joint__speech_kernel(x, w1, w2, g, w_f, w_g, w_o):
    return _fn(x, w1, w2, g, w_f, w_g, w_o)
```

```python
import functools
import numpy as np
import jax
import jax.numpy as jnp
from jax import lax
import jax.experimental.pallas as pl
import jax.experimental.pallas.tpu as pltpu

B, T, D, K, U = 2, 16000, 256, 31, 8
H = D // 2
T1, T2 = T // 2, T // 4
N = 64
HOP = 46
MC = 32
NB1 = 176
NB2 = NB1 // 2
NC1 = B * NB1 // MC
NC2 = 6
NJOB = NC1 + NC2
P1 = NB1 * HOP
P2 = NB2 * HOP
P3 = NB2 * HOP // 2
XR = 8 + B * P1 + 24
HR = MC * NC2 * HOP + 64
FR = MC * NC2 * HOP // 2
XOFF, HOFF, FOFF = 0, XR, XR + HR
SEQR = XR + HR + FR
WP = 260
WROWS = 3 * N * WP
SP = 36


def _coef_matrix():
    import ml_dtypes
    c = np.zeros((2, 2, N, 64), np.float64)
    k = np.arange(N)
    for n in range(62):
        tap, cc = n % 31, n // 31
        if tap % 2 == 0:
            j = tap // 2
            cp, cq = ((-1j, 1j) if cc == 0 else (1.0, -1.0))
        else:
            j = (tap + 1) // 2
            cp, cq = ((1.0, 1.0) if cc == 0 else (1j, 1j))
        e = np.exp(2j * np.pi * j * k / N)
        for which, coef in ((0, cp), (1, cq)):
            v = coef * e
            c[which, 0, :, n] = v.real
            c[which, 1, :, n] = v.imag
    c = c.reshape(2, 2, 4, 16, 64).transpose(0, 2, 1, 3, 4).reshape(4 * N, 64)
    hi_ = c.astype(np.float32).astype(ml_dtypes.bfloat16)
    lo_ = (c - hi_.astype(np.float64)).astype(np.float32).astype(ml_dtypes.bfloat16)
    return np.concatenate([hi_, lo_], axis=1)


COEF = np.concatenate([_coef_matrix(), np.zeros((16, H), _coef_matrix().dtype)], axis=0)
FINE = 1
FULLSTEP = 0
TT = 400
JSUB = 40
RS2 = float(np.sqrt(0.5))
HIMASK = np.uint32(0xFFFF0000)
OSCALE = 1.0 / (2 * N)
HS1 = 0.5 * OSCALE
S2 = OSCALE * HS1
HS2 = 0.5 * S2
GC0 = float(np.sqrt(2.0 / np.pi))
GC1 = 0.044715
f32, bf16, u32 = jnp.float32, jnp.bfloat16, jnp.uint32


def fft8(xr, xi):
    a0r, a0i = xr[0] + xr[4], xi[0] + xi[4]
    a1r, a1i = xr[0] - xr[4], xi[0] - xi[4]
    a2r, a2i = xr[2] + xr[6], xi[2] + xi[6]
    a3r, a3i = xr[2] - xr[6], xi[2] - xi[6]
    a4r, a4i = xr[1] + xr[5], xi[1] + xi[5]
    a5r, a5i = xr[1] - xr[5], xi[1] - xi[5]
    a6r, a6i = xr[3] + xr[7], xi[3] + xi[7]
    a7r, a7i = xr[3] - xr[7], xi[3] - xi[7]
    e0r, e0i = a0r + a2r, a0i + a2i
    e2r, e2i = a0r - a2r, a0i - a2i
    e1r, e1i = a1r + a3i, a1i - a3r
    e3r, e3i = a1r - a3i, a1i + a3r
    o0r, o0i = a4r + a6r, a4i + a6i
    o2r, o2i = a4r - a6r, a4i - a6i
    o1r, o1i = a5r + a7i, a5i - a7r
    o3r, o3i = a5r - a7i, a5i + a7r
    t1r, t1i = (o1r + o1i) * RS2, (o1i - o1r) * RS2
    u, v = (o3i - o3r) * RS2, (o3r + o3i) * RS2
    yr = [e0r + o0r, e1r + t1r, e2r + o2i, e3r + u, e0r - o0r, e1r - t1r, e2r - o2i, e3r - u]
    yi = [e0i + o0i, e1i + t1i, e2i - o2r, e3i - v, e0i - o0i, e1i - t1i, e2i + o2r, e3i + v]
    return yr, yi


def ifft8(xr, xi):
    yi, yr = fft8(xi, xr)
    return yr, yi


def idft4(xr, xi):
    s02r, s02i = xr[0] + xr[2], xi[0] + xi[2]
    d02r, d02i = xr[0] - xr[2], xi[0] - xi[2]
    s13r, s13i = xr[1] + xr[3], xi[1] + xi[3]
    d13r, d13i = xr[1] - xr[3], xi[1] - xi[3]
    yr = [s02r + s13r, d02r - d13i, s02r - s13r, d02r + d13i]
    yi = [s02i + s13i, d02i + d13r, s02i - s13i, d02i - d13r]
    return yr, yi


def tw(ar, ai, num, den):
    num = num % den
    if num == 0:
        return ar, ai
    if num * 4 == den:
        return -ai, ar
    if num * 2 == den:
        return -ar, -ai
    if num * 4 == 3 * den:
        return ai, -ar
    if (num * 8) % den == 0:
        q = num * 8 // den
        if q == 1:
            return (ar - ai) * RS2, (ar + ai) * RS2
        if q == 3:
            return (ar + ai) * (-RS2), (ar - ai) * RS2
        if q == 5:
            return (ai - ar) * RS2, (ar + ai) * (-RS2)
        return (ar + ai) * RS2, (ai - ar) * RS2
    c = float(np.cos(2 * np.pi * num / den))
    s = float(np.sin(2 * np.pi * num / den))
    return ar * c - ai * s, ar * s + ai * c


def gelu_consts(s):
    return float(GC0 * GC1 * s * s * s), float(GC0 * s)


def gelu_scaled(v, c3, c1):
    inner = v * ((v * v) * c3 + c1)
    return v * (jnp.tanh(inner) + 1.0)


def lo(w):
    return pltpu.bitcast(w << 16, f32)


def hi(w):
    return pltpu.bitcast(w & HIMASK, f32)


def pack2(a, b):
    return pltpu.pack_elementwise([a, b], packed_dtype=bf16)


class Gate:
    def __init__(self, zmask, lm=None, lv=None, every=None):
        self.z = zmask
        self.tok = None
        self.mtoks = []
        self.lm = 2 if lm is None else lm
        self.every = 1 if every is None else every
        self.cnt = 0
        self.vtoks = []
        self.lv = 8 if lv is None else lv

    def vpub(self, x):
        if self.lv > 0 and self.z is not None:
            self.vtoks.append(x)

    def mgate(self, w):
        if self.lv <= 0 or len(self.vtoks) < self.lv or self.vtoks[-self.lv] is None:
            return w
        x = self.vtoks[-self.lv]
        self.vtoks[-self.lv] = None
        tok = (x if x.dtype == u32 else pltpu.bitcast(x, u32)) & self.z
        head = w[0:8, :] | tok
        return jnp.concatenate([head, w[8:, :]], axis=0)

    def publish(self, g):
        if self.z is not None:
            self.mtoks.append(g[0:8, 0:H])

    def _tok(self):
        if self.z is None or len(self.mtoks) < self.lm:
            return None
        self.cnt += 1
        if self.cnt % self.every != 0:
            return None
        t = self.mtoks[-self.lm]
        if t.dtype != u32:
            t = pltpu.bitcast(t, u32) & self.z
            self.mtoks[-self.lm] = t
        return t

    def gate_w(self, w):
        t = self._tok()
        return w if t is None else (w | t)

    def gate_f(self, x):
        t = self._tok()
        if t is None:
            return x
        return pltpu.bitcast(pltpu.bitcast(x, u32) | t, f32)


def chain(gens):
    for g in gens:
        yield from g


def interleave(mgen, mtot, vgen, vtot, lead):
    if mgen is None:
        for _ in vgen:
            pass
        return
    if vgen is None:
        for _ in mgen:
            pass
        return
    m_done = v_done = 0.0
    m_alive = v_alive = True
    while m_alive or v_alive:
        pick_v = v_alive and (not m_alive or (v_done - lead) / max(vtot - lead, 1.0) <= m_done / mtot)
        try:
            if pick_v:
                v_done += next(vgen)
            else:
                m_done += next(mgen)
        except StopIteration:
            if pick_v:
                v_alive = False
            else:
                m_alive = False


def merge(a, at, b, bt, delay=0.0):
    ad = bd = 0.0
    aa = ba = True
    while aa or ba:
        fb = bd / bt
        fa = max(ad / at - delay, 0.0) / (1.0 - delay)
        pick_a = aa and (not ba or fa <= fb)
        try:
            c = next(a if pick_a else b)
        except StopIteration:
            if pick_a:
                aa = False
            else:
                ba = False
            continue
        if pick_a:
            ad += c
        else:
            bd += c
        yield c


def g_fwd_pass1(src, tr, ti, gate):
    for n2 in range(8):
        xr, xi = [], []
        for n1 in range(8):
            w = src[pl.ds(8 * n1 + n2, 8, stride=2 * HOP), :]
            if n1 == 0:
                w = gate.gate_w(w)
            xr.append(lo(w))
            xi.append(hi(w))
        ar, ai = fft8(xr, xi)
        if FINE:
            gate.vpub(ar[7])
            yield 19
            ar[1] = gate.gate_f(ar[1])
        for k1 in range(8):
            br, bi = tw(ar[k1], ai[k1], -n2 * k1, N)
            tr[k1, n2] = br
            ti[k1, n2] = bi
        gate.vpub(br)
        yield (10 if FINE else 29)


def g_fwd_pass2(tar, tai, tbr, tbi, zv, wrow0, gate):
    for k1 in range(8):
        la = [tar[k1, n] for n in range(8)]
        la[0] = gate.gate_f(la[0])
        ya_r, ya_i = fft8(la, [tai[k1, n] for n in range(8)])
        if FINE:
            gate.vpub(ya_i[7])
            yield 14
        lb = [tbr[k1, n] for n in range(8)]
        if FINE:
            lb[0] = gate.gate_f(lb[0])
        yb_r, yb_i = fft8(lb, [tbi[k1, n] for n in range(8)])
        for k2 in range(8):
            if FINE and k2 == 4:
                gate.vpub(yb_i[3])
                yield 14
                ya_r[4] = gate.gate_f(ya_r[4])
            k = k1 + 8 * k2
            zv[0, k, pl.ds(wrow0, 8), :] = pack2(ya_r[k2] + ya_i[k2], yb_r[k2] + yb_i[k2])
            zv[1, k, pl.ds(wrow0, 8), :] = pack2(ya_r[k2], yb_r[k2])
            zv[2, k, pl.ds(wrow0, 8), :] = pack2(ya_i[k2], yb_i[k2])
        gate.vpub(yb_i[7])
        yield (10 if FINE else 38)


def g_funit(seqw, src_row, col, zdst, wrow0, tb, z, gate):
    tar, tai, tbr, tbi = tb
    sub = seqw.at[col, pl.ds(src_row, 16 * HOP + 32), :]
    yield from g_fwd_pass1(sub, tar, tai, gate)
    yield from g_fwd_pass1(sub.at[pl.ds(HOP, 15 * HOP + 32), :], tbr, tbi, gate)
    views = [t.at[pl.ds(z, 8)] for t in tb]
    yield from g_fwd_pass2(*views, zdst.at[:, :, :, pl.ds(col * H, H)], wrow0, gate)


def g_mstep(k, zbuf, wf, ks, vr, vi, gate):
    kn = (N - k) & (N - 1)

    def dot(a, b, wi):
        l = pltpu.bitcast(jnp.concatenate([gate.mgate(a[:, 0:H]), a[:, H:D], b], axis=1), bf16)
        w = wf[pl.ds((wi * N + ks) * WP, D), :]
        g = jnp.dot(l, pltpu.bitcast(w, bf16), preferred_element_type=f32)
        gate.publish(g)
        return g
    g1 = dot(zbuf[0, k], zbuf[0, kn], 0)
    yield MC
    g2 = dot(zbuf[2, k], zbuf[1, kn], 1)
    vr[k] = g1 - g2
    yield MC
    g3 = dot(zbuf[1, k], zbuf[2, kn], 2)
    vi[k] = g1 - g3
    yield MC


def g_iunit(vr, vi, row0, ub, z, seqw, dst_row, gate, gc, doff=0):
    ur, ui = ub
    for k1 in range(8):
        xr = [vr[k1 + 8 * k2, pl.ds(row0, 8), :] for k2 in range(8)]
        xi = [vi[k1 + 8 * k2, pl.ds(row0, 8), :] for k2 in range(8)]
        xr[0] = gate.gate_f(xr[0])
        ar, ai = ifft8(xr, xi)
        if FINE:
            gate.vpub(ar[7])
            yield 15
            ar[1] = gate.gate_f(ar[1])
        for m2 in range(8):
            br, bi = tw(ar[m2], ai[m2], m2 * k1, N)
            ur[m2, k1] = br
            ui[m2, k1] = bi
        gate.vpub(br)
        yield (10 if FINE else 25)
    urz, uiz = ur.at[pl.ds(z, 8)], ui.at[pl.ds(z, 8)]
    n = 8 * HOP // 2
    dst = [seqw.at[c, pl.ds(dst_row, doff + n), :] for c in range(2)]
    for q in range(4):
        ys = []
        for m2 in (2 * q, 2 * q + 1):
            la = [urz[m2, k1] for k1 in range(8)]
            if m2 == 2 * q:
                la[0] = gate.gate_f(la[0])
            ys.append(ifft8(la, [uiz[m2, k1] for k1 in range(8)]))
        for m1 in range(6):
            m = 8 * m1 + 2 * q
            if m >= HOP:
                continue
            for part in range(2):
                va, vb = ys[0][part][m1], ys[1][part][m1]
                if m1 == 3 or (FINE and m1 in (1, 5) and part == 0):
                    va, vb = gate.gate_f(va), gate.gate_f(vb)
                a = gelu_scaled(va, *gc)
                b = gelu_scaled(vb, *gc)
                dst[part][pl.ds(doff + m // 2, 8, stride=HOP // 2), :] = pack2(a, b)
            if FINE and m1 == 0:
                gate.vpub(b)
                yield 30
            if m1 == 2:
                gate.vpub(b)
                yield (14 if FINE else 44)
            if FINE and m1 == 4:
                gate.vpub(b)
                yield 17
        gate.vpub(b)
        yield (14 if FINE else 31)


def g_wslab(ww, slab, wf, pb, sb, z, gate, whichs=(0, 1)):
    rows = pl.ds(pl.multiple_of(slab * 8, 8), 8)
    for j2 in range(4):
        raw = []
        for j1 in range(4):
            j = 4 * j1 + j2
            w0 = ww[0, 2 * j, rows, :]
            if j1 == 0:
                w0 = gate.gate_w(w0)
            w1_ = ww[1, 2 * j, rows, :]
            we = (ww[0, 2 * j - 1, rows, :], ww[1, 2 * j - 1, rows, :]) if j > 0 else None
            raw.append((w0, w1_, we))
        for ab, un in enumerate((lo, hi)):
            pq = []
            for (w0, w1_, we) in raw:
                vo0, vo1 = un(w0), un(w1_)
                if we is None:
                    pq.append(((vo1, -vo0), (-vo1, vo0)))
                else:
                    ve0, ve1 = un(we[0]), un(we[1])
                    pq.append(((ve0 + vo1, ve1 - vo0), (ve0 - vo1, ve1 + vo0)))
            for which in whichs:
                for r in range(4):
                    xr, xi = [], []
                    for j1 in range(4):
                        pr_, pi_ = pq[j1][which]
                        if j1 == 0 and (r > 0 or which > 0 or ab > 0):
                            pr_ = gate.gate_f(pr_)
                        a, b = tw(pr_, pi_, (4 * j1 + j2) * r, N)
                        xr.append(a)
                        xi.append(b)
                    yr, yi = idft4(xr, xi)
                    for k1 in range(4):
                        a, b = tw(yr[k1], yi[k1], j2 * k1, 16)
                        sb[which, 0, r * 16 + k1 * 4 + j2, ab] = a
                        sb[which, 1, r * 16 + k1 * 4 + j2, ab] = b
                    gate.vpub(b)
                    yield 12
    sbz = sb.at[pl.ds(z, 2)]
    for which in whichs:
        wv = wf.at[pl.ds(pl.multiple_of(slab * 8, 8), WROWS - 120), :]
        for r in range(4):
            for k1 in range(4):
                res = []
                for ab in range(2):
                    lr_ = [sbz[which, 0, r * 16 + k1 * 4 + j2, ab] for j2 in range(4)]
                    if ab == 0:
                        lr_[0] = gate.gate_f(lr_[0])
                    yr, yi = idft4(lr_, [sbz[which, 1, r * 16 + k1 * 4 + j2, ab] for j2 in range(4)])
                    if which:
                        res.append([(yi[k2], yi[k2] - yr[k2], yi[k2] + yr[k2]) for k2 in range(4)])
                    else:
                        res.append([(yr[k2], yr[k2] + yi[k2], yr[k2] - yi[k2]) for k2 in range(4)])
                for k2 in range(4):
                    k = 4 * (k1 + 4 * k2) + r
                    for t in range(3):
                        wv[pl.ds((t * N + k) * WP + which * H, 8), :] = pack2(res[0][k2][t], res[1][k2][t])
                gate.vpub(res[1][3][2])
                yield 16


def g_wpre(ww, slab, stg, gate):
    rows = pl.ds(pl.multiple_of(slab * 8, 8), 8)
    for p in range(31):
        na, nb = 2 * p, 2 * p + 1
        a = ww[na // 31, na % 31, rows, :]
        if p % 4 == 0:
            a = gate.gate_w(a)
        b = ww[nb // 31, nb % 31, rows, :]
        stg[0, pl.ds(p, 8, stride=SP), :] = pack2(lo(a), lo(b))
        o = pack2(hi(a), hi(b))
        stg[1, pl.ds(p, 8, stride=SP), :] = o
        if p % 4 == 3 or p == 30:
            gate.vpub(o)
            yield 7


def g_wmxu(stg, cmat, slab, wf, gate, whichs=(0, 1)):
    wv = wf.at[pl.ds(pl.multiple_of(slab * 8, 8), WROWS - 120), :]
    idx = 0
    for sp in range(4):
        for which in whichs:
            for kq in range(4):
                zi = pl.multiple_of((slab >> (16 + idx % 14)) * 8, 8)
                idx += 1
                cm = cmat.at[pl.ds(zi * 2, 4 * 64), :][pl.ds((which * 4 + kq) * 32, 32), :]
                sv = stg.at[:, pl.ds(zi, 8 * SP), :]
                rr = []
                for s_ in (2 * sp, 2 * sp + 1):
                    for ab in range(2):
                        r = pltpu.bitcast(sv[ab, pl.ds(s_ * SP, 32), :], bf16)
                        rr.append(jnp.concatenate([r, r], axis=0))
                g = jnp.dot(cm, jnp.concatenate(rr, axis=1), preferred_element_type=f32)
                gate.publish(g)
                yield 32
                for si, s_ in enumerate((2 * sp, 2 * sp + 1)):
                    for kg in range(2):
                        forms = []
                        for ab in range(2):
                            c0 = (2 * si + ab) * H
                            re = g[kg * 8:(kg + 1) * 8, c0:c0 + H]
                            im = g[16 + kg * 8:16 + (kg + 1) * 8, c0:c0 + H]
                            forms.append((im, im - re, im + re) if which else (re, re + im, re - im))
                        for t in range(3):
                            wv[pl.ds((t * N + 16 * kq + 8 * kg) * WP + which * H + s_, 8, stride=WP), :] = pack2(
                                forms[0][t], forms[1][t])


def _kernel(x_hbm, w1_hbm, w2_hbm, g_ref, wf_ref, wg_ref, wo_ref, cmat, o_hbm,
            seq, wraw1, wraw2, wfr1, wfr2, zA, zB, vAr, vAi, vBr, vBi,
            t0, t1, t2, t3, ur, ui, pb, sb, zz, obuf, sems, osems, w1sems, xsems, stg0, stg1, stg2):
    XQ = T // 4

    def xcopy(b, q, c):
        r0, n = (0, T) if q is None else (q * XQ, XQ)
        return pltpu.make_async_copy(
            x_hbm.at[b, pl.ds(r0, n), pl.ds(c * H, H)],
            seq.at[c, pl.ds(2 * XOFF + 16 + b * 2 * P1 + r0, n), :],
            xsems.at[(8 if q is None else 2 * q) + c])

    def xstart(b, q):
        for c in range(2):
            xcopy(b, q, c).start()

    def xwait(b, q):
        for c in range(2):
            xcopy(b, q, c).wait()
    WG = 4

    def w1copy(grp, c):
        rows = pl.ds(grp * (D // WG), D // WG)
        return pltpu.make_async_copy(w1_hbm.at[:, rows, pl.ds(c * H, H)], wraw1.at[c, :, rows, :], w1sems.at[grp * 2 + c])
    wcp1 = [w1copy(grp, c) for grp in range(WG) for c in range(2)]
    wcp2 = [pltpu.make_async_copy(w2_hbm.at[:, :, pl.ds(c * H, H)], wraw2.at[c], sems.at[6 + c]) for c in range(2)]
    for cp in wcp1:
        cp.start()
    xstart(0, 0)
    zero16 = lambda n: jnp.zeros((n, H), bf16)
    for c in range(2):
        seq[c, pl.ds(2 * XOFF, 16), :] = zero16(16)
        for b in range(B):
            n = 2 * P1 - T + (48 if b == B - 1 else 0)
            seq[c, pl.ds(2 * XOFF + 16 + b * 2 * P1 + T, n), :] = zero16(n)
        seq[c, pl.ds(2 * HOFF, 16), :] = zero16(16)
        n = 2 * HR - 16 - B * 2 * P2
        seq[c, pl.ds(2 * HOFF + 16 + B * 2 * P2, n), :] = zero16(n)
    zz[...] = jnp.zeros((8, H), u32)
    vBr[...] = jnp.zeros(vBr.shape, f32)
    vBi[...] = jnp.zeros(vBi.shape, f32)
    seqw = seq.bitcast(u32)
    tb, ub = (t0, t1, t2, t3), (ur, ui)
    nogate = Gate(None)

    ww1 = wraw1.bitcast(u32)
    ww2 = wraw2.bitcast(u32)

    W1MODE = 'mix'
    stgs = (stg0, stg1, stg2)
    for st in stgs:
        st[...] = jnp.zeros(st.shape, u32)

    def w1body(s, c):
        if W1MODE == 'v':
            for _ in g_wslab(ww1, s, wfr1, pb, sb, s >> 16, nogate):
                pass
        else:
            for _ in g_wpre(ww1, s, stg0, nogate):
                pass
            for _ in g_wmxu(stg0, cmat, s, wfr1, nogate):
                pass
        return c

    def w1group(grp):
        s0 = grp * 4
        gate = Gate(zz[...], lm=2, lv=0)
        vg = [g_wpre(ww1, s0 + a, stgs[a], gate) for a in range(3)]
        vg.append(g_wslab(ww1, s0 + 3, wfr1, pb, sb, s0 >> 16, gate))
        mg = [g_wmxu(stgs[a], cmat, s0 + a, wfr1, gate) for a in range(3)]
        interleave(chain(mg), 3 * 16 * 64, chain(vg), 3 * 56 + 64 * 12 + 32 * 16, 56.0)
    with jax.named_scope('ph_W1'):
        for grp in range(WG):
            for c in range(2):
                w1copy(grp, c).wait()
            if grp == 1:
                xstart(0, 1)
            if grp == 2:
                xstart(0, 2)
            if grp == 3:
                for cp in wcp2:
                    cp.start()
            n = D // 16 // WG
            if W1MODE == 'mix':
                def gb(u, c, grp=grp):
                    w1group(grp + (u >> 16))
                    return c
                lax.fori_loop(0, 1, gb, 0)
            else:
                lax.fori_loop(grp * n, (grp + 1) * n, w1body, 0)
    with jax.named_scope('ph_xwait0'):
        xwait(0, 0)
    xstart(0, 3)
    xstart(1, None)

    def src_row(job, g16):
        base = jnp.where(job < NC1, XOFF + job * (MC * HOP), HOFF + (job - NC1) * (MC * HOP))
        return pl.multiple_of(base + g16 * (16 * HOP), 32)

    def dst_row(job, g8):
        base = jnp.where(job < NC1, HOFF + 8 + job * (MC * HOP // 2), FOFF + (job - NC1) * (MC * HOP // 2))
        return pl.multiple_of(base + g8 * (8 * HOP // 2), 8)

    def f0body(g16, c):
        for col in range(2):
            for _ in g_funit(seqw, src_row(0, g16), col, zA, pl.multiple_of(g16 * 8, 8), tb, g16 >> 16, nogate):
                pass
        return c
    with jax.named_scope('ph_F0'):
        lax.fori_loop(0, MC // 16, f0body, 0)

    LEAD = 0.0

    def half_step(s, h, par, with_w):
        zM, zF = (zA, zB) if par == 0 else (zB, zA)
        vM, vI = ((vAr, vAi), (vBr, vBi)) if par == 0 else ((vBr, vBi), (vAr, vAi))
        wfr = wfr1
        z = h >> 16
        gate = Gate(zz[...])
        jf = jnp.minimum(s + 1, NJOB - 1)
        ji = jnp.maximum(s - 1, 0)
        ca, cb = gelu_consts(OSCALE), gelu_consts(S2)
        gc = (jnp.where(ji < NC1, ca[0], cb[0]).astype(f32), jnp.where(ji < NC1, ca[1], cb[1]).astype(f32))
        vg = []
        for col in range(2):
            vg.append(g_funit(seqw, src_row(jf, h), col, zF, pl.multiple_of(h * 8, 8), tb, z, gate))
            vg.append(g_iunit(vI[0], vI[1], pl.multiple_of(h * 16 + col * 8, 8), ub, z, seqw,
                              dst_row(ji, 2 * h + col), gate, gc))
        vtot = 2 * (16 * 29 + 8 * 38) + 2 * (8 * 25 + 4 * 75)
        if with_w:
            slab = 2 * (s - 1) + h
            if 1:
                vg.insert(0, g_wpre(ww2, slab, stg0, gate))
                vg.append(g_wslab(ww2, slab, wfr2, pb, sb, z, gate, whichs=(1,)))
                vtot += 56 + 32 * 14 + 16 * 16
            else:
                vg.append(g_wslab(ww2, slab, wfr2, pb, sb, z, gate))
                vtot += 64 * 12 + 32 * 16
        return zM, vM, gate, vg, vtot

    def run_half(s, h, par, with_w, wsel):
        zM, vM, gate, vg, vtot = half_step(s, h, par, with_w)
        wfr = wfr1 if wsel == 1 else wfr2
        wv = wfr.at[pl.ds(pl.multiple_of(h * (32 * WP), 8), WROWS - 32 * WP), :]
        mg = [g_mstep(h * 32 + a, zM, wv, a, vM[0], vM[1], gate) for a in range(32)]
        mgen, mtot = chain(mg), 32 * 3 * MC
        if with_w and 1:
            mgen = merge(mgen, mtot, g_wmxu(stg0, cmat, 2 * (s - 1) + h, wfr2, gate, whichs=(0,)), 16 * 32,
                         delay=0.15)
            mtot += 16 * 32
        interleave(mgen, mtot, chain(vg), vtot, LEAD)

    def run_full(s, par, with_w, wsel):
        zM, zF = (zA, zB) if par == 0 else (zB, zA)
        vM, vI = ((vAr, vAi), (vBr, vBi)) if par == 0 else ((vBr, vBi), (vAr, vAi))
        z = s >> 16
        gate = Gate(zz[...])
        jf = jnp.minimum(s + 1, NJOB - 1)
        ji = jnp.maximum(s - 1, 0)
        ca, cb = gelu_consts(OSCALE), gelu_consts(S2)
        gc = (jnp.where(ji < NC1, ca[0], cb[0]).astype(f32), jnp.where(ji < NC1, ca[1], cb[1]).astype(f32))
        vg = []
        vtot = 0
        dbase = pl.multiple_of(jnp.where(ji < NC1, HOFF + ji * (MC * HOP // 2),
                                         FOFF - 8 + (ji - NC1) * (MC * HOP // 2)), 8)
        for h in range(2):
            for col in range(2):
                vg.append(g_funit(seqw, src_row(jf, h), col, zF, pl.multiple_of(h * 8 + z * 32, 8), tb, z, gate))
                vg.append(g_iunit(vI[0], vI[1], pl.multiple_of(h * 16 + col * 8 + z * 32, 8), ub, z, seqw,
                                  dbase, gate, gc, doff=8 + (2 * h + col) * (8 * HOP // 2)))
            vtot += 2 * (16 * 29 + 8 * 38) + 2 * (8 * 25 + 4 * 75)
        wfr = wfr1 if wsel == 1 else wfr2
        mg = chain([g_mstep(a, zM, wfr, a, vM[0], vM[1], gate) for a in range(N)])
        mtot = N * 3 * MC
        vgen = chain(vg)
        if with_w:
            sa, sb_ = 2 * (s - 1), 2 * (s - 1) + 1
            vw = chain([g_wpre(ww2, sa, stg0, gate), g_wslab(ww2, sb_, wfr2, pb, sb, z, gate)])
            wt = 56 + 64 * 12 + 32 * 16
            if 0:
                vgen = merge(vw, wt, vgen, vtot)
            else:
                vgen = chain([g_wpre(ww2, sa, stg0, gate), vgen, g_wslab(ww2, sb_, wfr2, pb, sb, z, gate)])
            vtot += wt
            mg = merge(mg, mtot, g_wmxu(stg0, cmat, sa, wfr2, gate), 16 * 64, delay=0.15)
            mtot += 16 * 64
        interleave(mg, mtot, vgen, vtot, LEAD)

    def step(s, par, with_w, wsel):
        if (FULLSTEP and not with_w) or (with_w and 0):
            def sb_(u, c):
                run_full(s + (u >> 16), par, with_w, wsel)
                return c
            lax.fori_loop(0, 1, sb_, 0)
            return

        def hb(h, c):
            run_half(s, h, par, with_w, wsel)
            return c
        lax.fori_loop(0, 2, hb, 0)

    def pair_loop(p0, p1, with_w, wsel):
        def pb_(p, c):
            if with_w:
                @pl.when(p == 1)
                def _():
                    xwait(0, 3)

                @pl.when(p == 1)
                def _():
                    xwait(1, None)
                step(2 * p + 1, 1, with_w, wsel)
                step(2 * p + 2, 0, with_w, wsel)
                return c
            step(2 * p, 0, with_w, wsel)
            step(2 * p + 1, 1, with_w, wsel)
            return c
        lax.fori_loop(p0, p1, pb_, 0)

    with jax.named_scope('ph_c1w'):
        xwait(0, 1)
        step(jnp.int32(0), 0, False, 1)
        xwait(0, 2)
        for cp in wcp2:
            cp.wait()
        pair_loop(0, 4, True, 1)
    with jax.named_scope('ph_c1'):
        step(jnp.int32(9), 1, False, 1)
        step(jnp.int32(10), 0, False, 1)
    with jax.named_scope('ph_c2a'):
        step(jnp.int32(11), 1, False, 2)
    for c in range(2):
        for b in range(B):
            n = 2 * P2 - T1
            seq[c, pl.ds(2 * HOFF + 16 + b * 2 * P2 + T1, n), :] = zero16(n)
    with jax.named_scope('ph_c2b'):
        pair_loop(6, 8, False, 2)
        step(jnp.int32(16), 0, False, 2)

    def ilast(g8, c):
        for _ in g_iunit(vAr, vAi, pl.multiple_of(g8 * 8, 8), ub, g8 >> 16, seqw, dst_row(NJOB - 1, g8), nogate, gelu_consts(S2)):
            pass
        return c
    with jax.named_scope('ph_ilast'):
        lax.fori_loop(0, 2, ilast, 0)

    ntile = T2 // TT

    def ocopy(slot, b, t0_):
        return pltpu.make_async_copy(obuf.at[slot], o_hbm.at[b, pl.ds(t0_, TT)], osems.at[slot])

    for b in range(B):
        ge = jnp.dot(g_ref[b], wg_ref[...], preferred_element_type=f32)

        def jbody(i, c, b=b, ge=ge):
            step_ = b * ntile + i
            slot = step_ & 1
            t0_ = pl.multiple_of(i * TT, 16)

            @pl.when(step_ >= 2)
            def _():
                ocopy(slot, b, t0_).wait()
            frow = pl.multiple_of(2 * FOFF + b * 2 * P3 + i * TT, 16)
            f = jnp.concatenate([seq[0, pl.ds(frow, TT), :], seq[1, pl.ds(frow, TT), :]], axis=1)
            fe = jnp.dot(f, wf_ref[...], preferred_element_type=f32) * HS2
            for s_ in range(TT // JSUB):
                fes = fe[s_ * JSUB:(s_ + 1) * JSUB]
                j = jnp.tanh(fes[:, None, :] + ge[None, :, :]).reshape(JSUB * U, D).astype(bf16)
                o = jnp.dot(j, wo_ref[...], preferred_element_type=f32)
                obuf[slot, pl.ds(s_ * JSUB, JSUB)] = o.reshape(JSUB, U, D).astype(bf16)
            ocopy(slot, b, t0_).start()
            return c
        with jax.named_scope('ph_J'):
            lax.fori_loop(0, ntile, jbody, 0)
    with jax.named_scope('ph_tail'):
        for slot in range(2):
            ocopy(slot, 0, 0).wait()


def make(interpret=False):
    def fn(x, w1, w2, g, w_f, w_g, w_o):
        vm = pltpu.VMEM
        any_spec = pl.BlockSpec(memory_space=pl.ANY)
        vspec = pl.BlockSpec(memory_space=pltpu.VMEM)
        zsh = (3, N, MC // 2, D)
        vsh = (N, MC, H)
        return pl.pallas_call(
            _kernel,
            in_specs=[any_spec, any_spec, any_spec, vspec, vspec, vspec, vspec, vspec],
            out_specs=any_spec,
            out_shape=jax.ShapeDtypeStruct((B, T2, U, D), bf16),
            scratch_shapes=[
                vm((2, 2 * SEQR, H), bf16), vm((2, K, D, H), bf16), vm((2, K, D, H), bf16),
                vm((WROWS, H), u32), vm((WROWS, H), u32), vm(zsh, u32), vm(zsh, u32),
                vm(vsh, f32), vm(vsh, f32), vm(vsh, f32), vm(vsh, f32),
                vm((9, 8, 8, H), f32), vm((9, 8, 8, H), f32), vm((9, 8, 8, H), f32), vm((9, 8, 8, H), f32),
                vm((9, 8, 8, H), f32), vm((9, 8, 8, H), f32),
                vm((8, H), f32), vm((3, 2, 64, 2, 8, H), f32), vm((8, H), u32),
                vm((2, TT, U, D), bf16),
                pltpu.SemaphoreType.DMA((8,)), pltpu.SemaphoreType.DMA((2,)), pltpu.SemaphoreType.DMA((8,)),
                pltpu.SemaphoreType.DMA((10,)),
                vm((2, 8 * SP + 8, H), u32), vm((2, 8 * SP + 8, H), u32), vm((2, 8 * SP + 8, H), u32),
            ],
            compiler_params=pltpu.CompilerParams(vmem_limit_bytes=124 * 1024 * 1024),
            interpret=interpret,
            name="rnnt_fft3",
        )(x, w1, w2, g, w_f, w_g, w_o, jnp.asarray(COEF))
    return fn


_fn = make()


@jax.jit
def pallas_standalone__seq2seq_rnn_t_joint__speech_kernel(x, w1, w2, g, w_f, w_g, w_o):
    return _fn(x, w1, w2, g, w_f, w_g, w_o)
```

```python
import numpy as np
import jax
import jax.numpy as jnp
from jax import lax
import jax.experimental.pallas as pl
import jax.experimental.pallas.tpu as pltpu

B, T, D, K, U = 2, 16000, 256, 31, 8
H = D // 2
T1, T2 = T // 2, T // 4
N = 64
HOP = 46
MC = 32
NB1 = 176
NB2 = NB1 // 2
NC1 = B * NB1 // MC
NC2 = 6
NJOB = NC1 + NC2
P1 = NB1 * HOP
P2 = NB2 * HOP
P3 = NB2 * HOP // 2
XR = 8 + B * P1 + 24
HR = MC * NC2 * HOP + 64
FR = MC * NC2 * HOP // 2
XOFF, HOFF, FOFF = 0, XR, XR + HR
SEQR = XR + HR + FR
WP = 260
WROWS = 3 * N * WP
SP = 36


def _coef_matrix():
    import ml_dtypes
    c = np.zeros((2, 2, N, 64), np.float64)
    k = np.arange(N)
    for n in range(62):
        tap, cc = n % 31, n // 31
        if tap % 2 == 0:
            j = tap // 2
            cp, cq = ((-1j, 1j) if cc == 0 else (1.0, -1.0))
        else:
            j = (tap + 1) // 2
            cp, cq = ((1.0, 1.0) if cc == 0 else (1j, 1j))
        e = np.exp(2j * np.pi * j * k / N)
        for which, coef in ((0, cp), (1, cq)):
            v = coef * e
            c[which, 0, :, n] = v.real
            c[which, 1, :, n] = v.imag
    c = c.reshape(2, 2, 4, 16, 64).transpose(0, 2, 1, 3, 4).reshape(4 * N, 64)
    hi_ = c.astype(np.float32).astype(ml_dtypes.bfloat16)
    lo_ = (c - hi_.astype(np.float64)).astype(np.float32).astype(ml_dtypes.bfloat16)
    return np.concatenate([hi_, lo_], axis=1)


COEF = np.concatenate([_coef_matrix(), np.zeros((16, H), _coef_matrix().dtype)], axis=0)
TT = 400
JSUB = 40
RS2 = float(np.sqrt(0.5))
HIMASK = np.uint32(0xFFFF0000)
OSCALE = 1.0 / (2 * N)
HS1 = 0.5 * OSCALE
S2 = OSCALE * HS1
HS2 = 0.5 * S2
GC0 = float(np.sqrt(2.0 / np.pi))
GC1 = 0.044715
f32, bf16, u32 = jnp.float32, jnp.bfloat16, jnp.uint32


def fft8(xr, xi):
    a0r, a0i = xr[0] + xr[4], xi[0] + xi[4]
    a1r, a1i = xr[0] - xr[4], xi[0] - xi[4]
    a2r, a2i = xr[2] + xr[6], xi[2] + xi[6]
    a3r, a3i = xr[2] - xr[6], xi[2] - xi[6]
    a4r, a4i = xr[1] + xr[5], xi[1] + xi[5]
    a5r, a5i = xr[1] - xr[5], xi[1] - xi[5]
    a6r, a6i = xr[3] + xr[7], xi[3] + xi[7]
    a7r, a7i = xr[3] - xr[7], xi[3] - xi[7]
    e0r, e0i = a0r + a2r, a0i + a2i
    e2r, e2i = a0r - a2r, a0i - a2i
    e1r, e1i = a1r + a3i, a1i - a3r
    e3r, e3i = a1r - a3i, a1i + a3r
    o0r, o0i = a4r + a6r, a4i + a6i
    o2r, o2i = a4r - a6r, a4i - a6i
    o1r, o1i = a5r + a7i, a5i - a7r
    o3r, o3i = a5r - a7i, a5i + a7r
    t1r, t1i = (o1r + o1i) * RS2, (o1i - o1r) * RS2
    u, v = (o3i - o3r) * RS2, (o3r + o3i) * RS2
    yr = [e0r + o0r, e1r + t1r, e2r + o2i, e3r + u, e0r - o0r, e1r - t1r, e2r - o2i, e3r - u]
    yi = [e0i + o0i, e1i + t1i, e2i - o2r, e3i - v, e0i - o0i, e1i - t1i, e2i + o2r, e3i + v]
    return yr, yi


def ifft8(xr, xi):
    yi, yr = fft8(xi, xr)
    return yr, yi


def idft4(xr, xi):
    s02r, s02i = xr[0] + xr[2], xi[0] + xi[2]
    d02r, d02i = xr[0] - xr[2], xi[0] - xi[2]
    s13r, s13i = xr[1] + xr[3], xi[1] + xi[3]
    d13r, d13i = xr[1] - xr[3], xi[1] - xi[3]
    yr = [s02r + s13r, d02r - d13i, s02r - s13r, d02r + d13i]
    yi = [s02i + s13i, d02i + d13r, s02i - s13i, d02i - d13r]
    return yr, yi


def tw(ar, ai, num, den):
    num = num % den
    if num == 0:
        return ar, ai
    if num * 4 == den:
        return -ai, ar
    if num * 2 == den:
        return -ar, -ai
    if num * 4 == 3 * den:
        return ai, -ar
    if (num * 8) % den == 0:
        q = num * 8 // den
        if q == 1:
            return (ar - ai) * RS2, (ar + ai) * RS2
        if q == 3:
            return (ar + ai) * (-RS2), (ar - ai) * RS2
        if q == 5:
            return (ai - ar) * RS2, (ar + ai) * (-RS2)
        return (ar + ai) * RS2, (ai - ar) * RS2
    c = float(np.cos(2 * np.pi * num / den))
    s = float(np.sin(2 * np.pi * num / den))
    return ar * c - ai * s, ar * s + ai * c


def gelu_consts(s):
    return float(GC0 * GC1 * s * s * s), float(GC0 * s)


def gelu_scaled(v, c3, c1):
    inner = v * ((v * v) * c3 + c1)
    return v * (jnp.tanh(inner) + 1.0)


def lo(w):
    return pltpu.bitcast(w << 16, f32)


def hi(w):
    return pltpu.bitcast(w & HIMASK, f32)


def pack2(a, b):
    return pltpu.pack_elementwise([a, b], packed_dtype=bf16)


class Gate:
    def __init__(self, zmask, lm=2, lv=8):
        self.z = zmask
        self.lm, self.lv = lm, lv
        self.mtoks, self.vtoks = [], []

    def vpub(self, x):
        if self.lv > 0 and self.z is not None:
            self.vtoks.append(x)

    def mgate(self, w):
        if self.lv <= 0 or len(self.vtoks) < self.lv or self.vtoks[-self.lv] is None:
            return w
        x = self.vtoks[-self.lv]
        self.vtoks[-self.lv] = None
        tok = (x if x.dtype == u32 else pltpu.bitcast(x, u32)) & self.z
        head = w[0:8, :] | tok
        return jnp.concatenate([head, w[8:, :]], axis=0)

    def publish(self, g):
        if self.z is not None:
            self.mtoks.append(g[0:8, 0:H])

    def _tok(self):
        if self.z is None or len(self.mtoks) < self.lm:
            return None
        t = self.mtoks[-self.lm]
        if t.dtype != u32:
            t = pltpu.bitcast(t, u32) & self.z
            self.mtoks[-self.lm] = t
        return t

    def gate_w(self, w):
        t = self._tok()
        return w if t is None else (w | t)

    def gate_f(self, x):
        t = self._tok()
        if t is None:
            return x
        return pltpu.bitcast(pltpu.bitcast(x, u32) | t, f32)


def chain(gens):
    for g in gens:
        yield from g


def interleave(mgen, mtot, vgen, vtot, lead):
    if mgen is None:
        for _ in vgen:
            pass
        return
    if vgen is None:
        for _ in mgen:
            pass
        return
    m_done = v_done = 0.0
    m_alive = v_alive = True
    while m_alive or v_alive:
        pick_v = v_alive and (not m_alive or (v_done - lead) / max(vtot - lead, 1.0) <= m_done / mtot)
        try:
            if pick_v:
                v_done += next(vgen)
            else:
                m_done += next(mgen)
        except StopIteration:
            if pick_v:
                v_alive = False
            else:
                m_alive = False


def merge(a, at, b, bt, delay=0.0):
    ad = bd = 0.0
    aa = ba = True
    while aa or ba:
        fb = bd / bt
        fa = max(ad / at - delay, 0.0) / (1.0 - delay)
        pick_a = aa and (not ba or fa <= fb)
        try:
            c = next(a if pick_a else b)
        except StopIteration:
            if pick_a:
                aa = False
            else:
                ba = False
            continue
        if pick_a:
            ad += c
        else:
            bd += c
        yield c


def g_fwd_pass1(src, tr, ti, gate):
    for n2 in range(8):
        xr, xi = [], []
        for n1 in range(8):
            w = src[pl.ds(8 * n1 + n2, 8, stride=2 * HOP), :]
            if n1 == 0:
                w = gate.gate_w(w)
            xr.append(lo(w))
            xi.append(hi(w))
        ar, ai = fft8(xr, xi)
        gate.vpub(ar[7])
        yield 19
        ar[1] = gate.gate_f(ar[1])
        for k1 in range(8):
            br, bi = tw(ar[k1], ai[k1], -n2 * k1, N)
            tr[k1, n2] = br
            ti[k1, n2] = bi
        gate.vpub(br)
        yield 10


def g_fwd_pass2(tar, tai, tbr, tbi, zv, wrow0, gate):
    for k1 in range(8):
        la = [tar[k1, n] for n in range(8)]
        la[0] = gate.gate_f(la[0])
        ya_r, ya_i = fft8(la, [tai[k1, n] for n in range(8)])
        gate.vpub(ya_i[7])
        yield 14
        lb = [tbr[k1, n] for n in range(8)]
        lb[0] = gate.gate_f(lb[0])
        yb_r, yb_i = fft8(lb, [tbi[k1, n] for n in range(8)])
        for k2 in range(8):
            if k2 == 4:
                gate.vpub(yb_i[3])
                yield 14
                ya_r[4] = gate.gate_f(ya_r[4])
            k = k1 + 8 * k2
            zv[0, k, pl.ds(wrow0, 8), :] = pack2(ya_r[k2] + ya_i[k2], yb_r[k2] + yb_i[k2])
            zv[1, k, pl.ds(wrow0, 8), :] = pack2(ya_r[k2], yb_r[k2])
            zv[2, k, pl.ds(wrow0, 8), :] = pack2(ya_i[k2], yb_i[k2])
        gate.vpub(yb_i[7])
        yield 10


def g_funit(seqw, src_row, col, zdst, wrow0, tb, z, gate):
    tar, tai, tbr, tbi = tb
    sub = seqw.at[col, pl.ds(src_row, 16 * HOP + 32), :]
    yield from g_fwd_pass1(sub, tar, tai, gate)
    yield from g_fwd_pass1(sub.at[pl.ds(HOP, 15 * HOP + 32), :], tbr, tbi, gate)
    views = [t.at[pl.ds(z, 8)] for t in tb]
    yield from g_fwd_pass2(*views, zdst.at[:, :, :, pl.ds(col * H, H)], wrow0, gate)


def g_mstep(k, zbuf, wf, ks, vr, vi, gate):
    kn = (N - k) & (N - 1)

    def dot(a, b, wi):
        l = pltpu.bitcast(jnp.concatenate([gate.mgate(a[:, 0:H]), a[:, H:D], b], axis=1), bf16)
        w = wf[pl.ds((wi * N + ks) * WP, D), :]
        g = jnp.dot(l, pltpu.bitcast(w, bf16), preferred_element_type=f32)
        gate.publish(g)
        return g
    g1 = dot(zbuf[0, k], zbuf[0, kn], 0)
    yield MC
    g2 = dot(zbuf[2, k], zbuf[1, kn], 1)
    vr[k] = g1 - g2
    yield MC
    g3 = dot(zbuf[1, k], zbuf[2, kn], 2)
    vi[k] = g1 - g3
    yield MC


def g_iunit(vr, vi, row0, ub, z, seqw, dst_row, gate, gc):
    ur, ui = ub
    for k1 in range(8):
        xr = [vr[k1 + 8 * k2, pl.ds(row0, 8), :] for k2 in range(8)]
        xi = [vi[k1 + 8 * k2, pl.ds(row0, 8), :] for k2 in range(8)]
        xr[0] = gate.gate_f(xr[0])
        ar, ai = ifft8(xr, xi)
        gate.vpub(ar[7])
        yield 15
        ar[1] = gate.gate_f(ar[1])
        for m2 in range(8):
            br, bi = tw(ar[m2], ai[m2], m2 * k1, N)
            ur[m2, k1] = br
            ui[m2, k1] = bi
        gate.vpub(br)
        yield 10
    urz, uiz = ur.at[pl.ds(z, 8)], ui.at[pl.ds(z, 8)]
    n = 8 * HOP // 2
    dst = [seqw.at[c, pl.ds(dst_row, n), :] for c in range(2)]
    for q in range(4):
        ys = []
        for m2 in (2 * q, 2 * q + 1):
            la = [urz[m2, k1] for k1 in range(8)]
            if m2 == 2 * q:
                la[0] = gate.gate_f(la[0])
            ys.append(ifft8(la, [uiz[m2, k1] for k1 in range(8)]))
        for m1 in range(6):
            m = 8 * m1 + 2 * q
            if m >= HOP:
                continue
            for part in range(2):
                va, vb = ys[0][part][m1], ys[1][part][m1]
                if m1 == 3 or (m1 in (1, 5) and part == 0):
                    va, vb = gate.gate_f(va), gate.gate_f(vb)
                a = gelu_scaled(va, *gc)
                b = gelu_scaled(vb, *gc)
                dst[part][pl.ds(m // 2, 8, stride=HOP // 2), :] = pack2(a, b)
            if m1 == 0:
                gate.vpub(b)
                yield 30
            if m1 == 2:
                gate.vpub(b)
                yield 14
            if m1 == 4:
                gate.vpub(b)
                yield 17
        gate.vpub(b)
        yield 14


def g_wslab(ww, slab, wf, sb, z, gate, whichs=(0, 1)):
    rows = pl.ds(pl.multiple_of(slab * 8, 8), 8)
    for j2 in range(4):
        raw = []
        for j1 in range(4):
            j = 4 * j1 + j2
            w0 = ww[0, 2 * j, rows, :]
            if j1 == 0:
                w0 = gate.gate_w(w0)
            w1_ = ww[1, 2 * j, rows, :]
            we = (ww[0, 2 * j - 1, rows, :], ww[1, 2 * j - 1, rows, :]) if j > 0 else None
            raw.append((w0, w1_, we))
        for ab, un in enumerate((lo, hi)):
            pq = []
            for (w0, w1_, we) in raw:
                vo0, vo1 = un(w0), un(w1_)
                if we is None:
                    pq.append(((vo1, -vo0), (-vo1, vo0)))
                else:
                    ve0, ve1 = un(we[0]), un(we[1])
                    pq.append(((ve0 + vo1, ve1 - vo0), (ve0 - vo1, ve1 + vo0)))
            for which in whichs:
                for r in range(4):
                    xr, xi = [], []
                    for j1 in range(4):
                        pr_, pi_ = pq[j1][which]
                        if j1 == 0 and (r > 0 or which > 0 or ab > 0):
                            pr_ = gate.gate_f(pr_)
                        a, b = tw(pr_, pi_, (4 * j1 + j2) * r, N)
                        xr.append(a)
                        xi.append(b)
                    yr, yi = idft4(xr, xi)
                    for k1 in range(4):
                        a, b = tw(yr[k1], yi[k1], j2 * k1, 16)
                        sb[which, 0, r * 16 + k1 * 4 + j2, ab] = a
                        sb[which, 1, r * 16 + k1 * 4 + j2, ab] = b
                    gate.vpub(b)
                    yield 12
    sbz = sb.at[pl.ds(z, 2)]
    for which in whichs:
        wv = wf.at[pl.ds(pl.multiple_of(slab * 8, 8), WROWS - 120), :]
        for r in range(4):
            for k1 in range(4):
                res = []
                for ab in range(2):
                    lr_ = [sbz[which, 0, r * 16 + k1 * 4 + j2, ab] for j2 in range(4)]
                    if ab == 0:
                        lr_[0] = gate.gate_f(lr_[0])
                    yr, yi = idft4(lr_, [sbz[which, 1, r * 16 + k1 * 4 + j2, ab] for j2 in range(4)])
                    if which:
                        res.append([(yi[k2], yi[k2] - yr[k2], yi[k2] + yr[k2]) for k2 in range(4)])
                    else:
                        res.append([(yr[k2], yr[k2] + yi[k2], yr[k2] - yi[k2]) for k2 in range(4)])
                for k2 in range(4):
                    k = 4 * (k1 + 4 * k2) + r
                    for t in range(3):
                        wv[pl.ds((t * N + k) * WP + which * H, 8), :] = pack2(res[0][k2][t], res[1][k2][t])
                gate.vpub(res[1][3][2])
                yield 16


def g_wpre(ww, slab, stg, gate):
    rows = pl.ds(pl.multiple_of(slab * 8, 8), 8)
    for p in range(31):
        na, nb = 2 * p, 2 * p + 1
        a = ww[na // 31, na % 31, rows, :]
        if p % 4 == 0:
            a = gate.gate_w(a)
        b = ww[nb // 31, nb % 31, rows, :]
        stg[0, pl.ds(p, 8, stride=SP), :] = pack2(lo(a), lo(b))
        o = pack2(hi(a), hi(b))
        stg[1, pl.ds(p, 8, stride=SP), :] = o
        if p % 4 == 3 or p == 30:
            gate.vpub(o)
            yield 7


def g_wmxu(stg, cmat, slab, wf, gate, whichs=(0, 1)):
    wv = wf.at[pl.ds(pl.multiple_of(slab * 8, 8), WROWS - 120), :]
    idx = 0
    for sp in range(4):
        for which in whichs:
            for kq in range(4):
                zi = pl.multiple_of((slab >> (16 + idx % 14)) * 8, 8)
                idx += 1
                cm = cmat.at[pl.ds(zi * 2, 4 * 64), :][pl.ds((which * 4 + kq) * 32, 32), :]
                sv = stg.at[:, pl.ds(zi, 8 * SP), :]
                rr = []
                for s_ in (2 * sp, 2 * sp + 1):
                    for ab in range(2):
                        r = pltpu.bitcast(sv[ab, pl.ds(s_ * SP, 32), :], bf16)
                        rr.append(jnp.concatenate([r, r], axis=0))
                g = jnp.dot(cm, jnp.concatenate(rr, axis=1), preferred_element_type=f32)
                gate.publish(g)
                yield 32
                for si, s_ in enumerate((2 * sp, 2 * sp + 1)):
                    for kg in range(2):
                        forms = []
                        for ab in range(2):
                            c0 = (2 * si + ab) * H
                            re = g[kg * 8:(kg + 1) * 8, c0:c0 + H]
                            im = g[16 + kg * 8:16 + (kg + 1) * 8, c0:c0 + H]
                            forms.append((im, im - re, im + re) if which else (re, re + im, re - im))
                        for t in range(3):
                            wv[pl.ds((t * N + 16 * kq + 8 * kg) * WP + which * H + s_, 8, stride=WP), :] = pack2(
                                forms[0][t], forms[1][t])


def _kernel(x_hbm, w1_hbm, w2_hbm, g_ref, wf_ref, wg_ref, wo_ref, cmat, o_hbm,
            seq, wraw1, wraw2, wfr1, wfr2, zA, zB, vAr, vAi, vBr, vBi,
            t0, t1, t2, t3, ur, ui, sb, zz, obuf, sems, osems, w1sems, xsems, stg0, stg1, stg2):
    XQ = T // 4

    def xcopy(b, q, c):
        r0, n = (0, T) if q is None else (q * XQ, XQ)
        return pltpu.make_async_copy(
            x_hbm.at[b, pl.ds(r0, n), pl.ds(c * H, H)],
            seq.at[c, pl.ds(2 * XOFF + 16 + b * 2 * P1 + r0, n), :],
            xsems.at[(8 if q is None else 2 * q) + c])

    def xstart(b, q):
        for c in range(2):
            xcopy(b, q, c).start()

    def xwait(b, q):
        for c in range(2):
            xcopy(b, q, c).wait()
    WG = 4

    def w1copy(grp, c):
        rows = pl.ds(grp * (D // WG), D // WG)
        return pltpu.make_async_copy(w1_hbm.at[:, rows, pl.ds(c * H, H)], wraw1.at[c, :, rows, :], w1sems.at[grp * 2 + c])
    wcp1 = [w1copy(grp, c) for grp in range(WG) for c in range(2)]
    wcp2 = [pltpu.make_async_copy(w2_hbm.at[:, :, pl.ds(c * H, H)], wraw2.at[c], sems.at[6 + c]) for c in range(2)]
    for cp in wcp1:
        cp.start()
    xstart(0, 0)
    zero16 = lambda n: jnp.zeros((n, H), bf16)
    for c in range(2):
        seq[c, pl.ds(2 * XOFF, 16), :] = zero16(16)
        for b in range(B):
            n = 2 * P1 - T + (48 if b == B - 1 else 0)
            seq[c, pl.ds(2 * XOFF + 16 + b * 2 * P1 + T, n), :] = zero16(n)
        seq[c, pl.ds(2 * HOFF, 16), :] = zero16(16)
        n = 2 * HR - 16 - B * 2 * P2
        seq[c, pl.ds(2 * HOFF + 16 + B * 2 * P2, n), :] = zero16(n)
    zz[...] = jnp.zeros((8, H), u32)
    vBr[...] = jnp.zeros(vBr.shape, f32)
    vBi[...] = jnp.zeros(vBi.shape, f32)
    seqw = seq.bitcast(u32)
    tb, ub = (t0, t1, t2, t3), (ur, ui)
    nogate = Gate(None)

    ww1 = wraw1.bitcast(u32)
    ww2 = wraw2.bitcast(u32)

    stgs = (stg0, stg1, stg2)
    for st in stgs:
        st[...] = jnp.zeros(st.shape, u32)

    def w1group(grp):
        s0 = grp * 4
        gate = Gate(zz[...], lm=2, lv=0)
        vg = [g_wpre(ww1, s0 + a, stgs[a], gate) for a in range(3)]
        vg.append(g_wslab(ww1, s0 + 3, wfr1, sb, s0 >> 16, gate))
        mg = [g_wmxu(stgs[a], cmat, s0 + a, wfr1, gate) for a in range(3)]
        interleave(chain(mg), 3 * 16 * 64, chain(vg), 3 * 56 + 64 * 12 + 32 * 16, 56.0)

    for grp in range(WG):
        for c in range(2):
            w1copy(grp, c).wait()
        if grp == 1:
            xstart(0, 1)
        if grp == 2:
            xstart(0, 2)
        if grp == 3:
            for cp in wcp2:
                cp.start()

        def gb(u, c, grp=grp):
            w1group(grp + (u >> 16))
            return c
        lax.fori_loop(0, 1, gb, 0)
    xwait(0, 0)
    xstart(0, 3)
    xstart(1, None)

    def src_row(job, g16):
        base = jnp.where(job < NC1, XOFF + job * (MC * HOP), HOFF + (job - NC1) * (MC * HOP))
        return pl.multiple_of(base + g16 * (16 * HOP), 32)

    def dst_row(job, g8):
        base = jnp.where(job < NC1, HOFF + 8 + job * (MC * HOP // 2), FOFF + (job - NC1) * (MC * HOP // 2))
        return pl.multiple_of(base + g8 * (8 * HOP // 2), 8)

    def f0body(g16, c):
        for col in range(2):
            for _ in g_funit(seqw, src_row(0, g16), col, zA, pl.multiple_of(g16 * 8, 8), tb, g16 >> 16, nogate):
                pass
        return c
    lax.fori_loop(0, MC // 16, f0body, 0)

    def run_half(s, h, par, with_w, wsel):
        zM, zF = (zA, zB) if par == 0 else (zB, zA)
        vM, vI = ((vAr, vAi), (vBr, vBi)) if par == 0 else ((vBr, vBi), (vAr, vAi))
        z = h >> 16
        gate = Gate(zz[...], lv=10 if with_w else 8)
        jf = jnp.minimum(s + 1, NJOB - 1)
        ji = jnp.maximum(s - 1, 0)
        ca, cb = gelu_consts(OSCALE), gelu_consts(S2)
        gc = (jnp.where(ji < NC1, ca[0], cb[0]).astype(f32), jnp.where(ji < NC1, ca[1], cb[1]).astype(f32))
        vg = []
        for col in range(2):
            vg.append(g_iunit(vI[0], vI[1], pl.multiple_of(h * 16 + col * 8, 8), ub, z, seqw,
                              dst_row(ji, 2 * h + col), gate, gc))
            vg.append(g_funit(seqw, src_row(jf, h), col, zF, pl.multiple_of(h * 8, 8), tb, z, gate))
        vtot = 2 * (16 * 29 + 8 * 38) + 2 * (8 * 25 + 4 * 75)
        if with_w:
            slab = 2 * (s - 1) + h
            vg.insert(0, g_wpre(ww2, slab, stg0, gate))
            vg.append(g_wslab(ww2, slab, wfr2, sb, z, gate, whichs=(1,)))
            vtot += 56 + 32 * 14 + 16 * 16
        wfr = wfr1 if wsel == 1 else wfr2
        wv = wfr.at[pl.ds(pl.multiple_of(h * (32 * WP), 8), WROWS - 32 * WP), :]
        mg = [g_mstep(h * 32 + a, zM, wv, a, vM[0], vM[1], gate) for a in range(32)]
        mgen, mtot = chain(mg), 32 * 3 * MC
        if with_w:
            mgen = merge(mgen, mtot, g_wmxu(stg0, cmat, 2 * (s - 1) + h, wfr2, gate, whichs=(0,)), 16 * 32,
                         delay=0.15)
            mtot += 16 * 32
        interleave(mgen, mtot, chain(vg), vtot, 0.0)

    def step(s, par, with_w, wsel):
        def hb(h, c):
            run_half(s, h, par, with_w, wsel)
            return c
        lax.fori_loop(0, 2, hb, 0)

    def pair_loop(p0, p1, with_w, wsel):
        def pb_(p, c):
            if with_w:
                @pl.when(p == 1)
                def _():
                    xwait(0, 3)

                @pl.when(p == 1)
                def _():
                    xwait(1, None)
                step(2 * p + 1, 1, with_w, wsel)
                step(2 * p + 2, 0, with_w, wsel)
                return c
            step(2 * p, 0, with_w, wsel)
            step(2 * p + 1, 1, with_w, wsel)
            return c
        lax.fori_loop(p0, p1, pb_, 0)

    xwait(0, 1)
    step(jnp.int32(0), 0, False, 1)
    xwait(0, 2)
    for cp in wcp2:
        cp.wait()
    pair_loop(0, 4, True, 1)
    step(jnp.int32(9), 1, False, 1)
    step(jnp.int32(10), 0, False, 1)
    step(jnp.int32(11), 1, False, 2)
    for c in range(2):
        for b in range(B):
            n = 2 * P2 - T1
            seq[c, pl.ds(2 * HOFF + 16 + b * 2 * P2 + T1, n), :] = zero16(n)
    pair_loop(6, 8, False, 2)
    step(jnp.int32(16), 0, False, 2)

    def ilast(g8, c):
        for _ in g_iunit(vAr, vAi, pl.multiple_of(g8 * 8, 8), ub, g8 >> 16, seqw, dst_row(NJOB - 1, g8), nogate, gelu_consts(S2)):
            pass
        return c
    lax.fori_loop(0, 2, ilast, 0)

    ntile = T2 // TT

    def ocopy(slot, b, t0_):
        return pltpu.make_async_copy(obuf.at[slot], o_hbm.at[b, pl.ds(t0_, TT)], osems.at[slot])

    for b in range(B):
        ge = jnp.dot(g_ref[b], wg_ref[...], preferred_element_type=f32)

        def jbody(i, c, b=b, ge=ge):
            step_ = b * ntile + i
            slot = step_ & 1
            t0_ = pl.multiple_of(i * TT, 16)

            @pl.when(step_ >= 2)
            def _():
                ocopy(slot, b, t0_).wait()
            frow = pl.multiple_of(2 * FOFF + b * 2 * P3 + i * TT, 16)
            f = jnp.concatenate([seq[0, pl.ds(frow, TT), :], seq[1, pl.ds(frow, TT), :]], axis=1)
            fe = jnp.dot(f, wf_ref[...], preferred_element_type=f32) * HS2
            for s_ in range(TT // JSUB):
                fes = fe[s_ * JSUB:(s_ + 1) * JSUB]
                j = jnp.tanh(fes[:, None, :] + ge[None, :, :]).reshape(JSUB * U, D).astype(bf16)
                o = jnp.dot(j, wo_ref[...], preferred_element_type=f32)
                obuf[slot, pl.ds(s_ * JSUB, JSUB)] = o.reshape(JSUB, U, D).astype(bf16)
            ocopy(slot, b, t0_).start()
            return c
        lax.fori_loop(0, ntile, jbody, 0)
    for slot in range(2):
        ocopy(slot, 0, 0).wait()


def make(interpret=False):
    def fn(x, w1, w2, g, w_f, w_g, w_o):
        vm = pltpu.VMEM
        any_spec = pl.BlockSpec(memory_space=pl.ANY)
        vspec = pl.BlockSpec(memory_space=pltpu.VMEM)
        zsh = (3, N, MC // 2, D)
        vsh = (N, MC, H)
        return pl.pallas_call(
            _kernel,
            in_specs=[any_spec, any_spec, any_spec, vspec, vspec, vspec, vspec, vspec],
            out_specs=any_spec,
            out_shape=jax.ShapeDtypeStruct((B, T2, U, D), bf16),
            scratch_shapes=[
                vm((2, 2 * SEQR, H), bf16), vm((2, K, D, H), bf16), vm((2, K, D, H), bf16),
                vm((WROWS, H), u32), vm((WROWS, H), u32), vm(zsh, u32), vm(zsh, u32),
                vm(vsh, f32), vm(vsh, f32), vm(vsh, f32), vm(vsh, f32),
                vm((9, 8, 8, H), f32), vm((9, 8, 8, H), f32), vm((9, 8, 8, H), f32), vm((9, 8, 8, H), f32),
                vm((9, 8, 8, H), f32), vm((9, 8, 8, H), f32),
                vm((3, 2, 64, 2, 8, H), f32), vm((8, H), u32),
                vm((2, TT, U, D), bf16),
                pltpu.SemaphoreType.DMA((8,)), pltpu.SemaphoreType.DMA((2,)), pltpu.SemaphoreType.DMA((8,)),
                pltpu.SemaphoreType.DMA((10,)),
                vm((2, 8 * SP + 8, H), u32), vm((2, 8 * SP + 8, H), u32), vm((2, 8 * SP + 8, H), u32),
            ],
            compiler_params=pltpu.CompilerParams(vmem_limit_bytes=124 * 1024 * 1024),
            interpret=interpret,
            name="rnnt_joint_fft",
        )(x, w1, w2, g, w_f, w_g, w_o, jnp.asarray(COEF))
    return fn


_fn = make()


@jax.jit
def pallas_standalone__seq2seq_rnn_t_joint__speech_kernel(x, w1, w2, g, w_f, w_g, w_o):
    return _fn(x, w1, w2, g, w_f, w_g, w_o)
```
